```python
import os as _os
_os.environ.setdefault("JAX_PLATFORMS", "cpu")
import jax
import jax.numpy as jnp

def _softmax(x, axis=-1):
    return jax.nn.softmax(x, axis=axis)
def _gelu(x):
    return jax.nn.gelu(x, approximate=True)
def _silu(x):
    return jax.nn.silu(x)
def _sigmoid(x):
    return jax.nn.sigmoid(x)
def _layernorm(x, axis=-1, eps=1e-5):
    m = jnp.mean(x, axis=axis, keepdims=True)
    v = jnp.var(x, axis=axis, keepdims=True)
    return (x - m) / jnp.sqrt(v + eps)
def _scatter_add(tgt, idx, src, axis=0):
    return tgt.at[idx].add(src)
def _segment_sum(src, seg, n):
    return jax.ops.segment_sum(src, seg, n)
class _Rng:
    def __init__(self, key):
        self._k = key
    def _next(self):
        self._k, sub = jax.random.split(self._k)
        return sub
    def normal(self, shape):
        return jax.random.normal(self._next(), shape, dtype=jnp.bfloat16)
    def randint(self, lo, hi, shape):
        return jax.random.randint(self._next(), shape, lo, hi, dtype=jnp.int32)
    def uniform(self, shape, lo=0.0, hi=1.0):
        return jax.random.uniform(self._next(), shape, jnp.bfloat16, lo, hi)
    def permutation(self, n):
        return jax.random.permutation(self._next(), n)


kernel_name = 'concat_heads__softmax_full_mha__grouped_kv_mqa__prompt'

def setup_inputs():
    _rng = _Rng(jax.random.key(int.from_bytes(__import__("os").urandom(4), "little")))
    _w = (lambda a: (lambda t: t.astype(jnp.bfloat16) if jnp.issubdtype(t.dtype, jnp.floating) else t)(jnp.asarray(a)))
    def _A_setup():
        B, S, D = 1, 2048, 640
        return {
            "x": _w((lambda *s: _rng.normal(s) * 0.1)(B, S, D)),
            "wqkv": _w((lambda *s: _rng.normal(s) * 0.1)(D, 3 * D)),
            "wo": _w((lambda *s: _rng.normal(s) * 0.05)(D, D)),
        }
    _A_in = _A_setup()

    def _B_setup():
        B, S, D, H = 1, 2048, 640, 32
        Dh = D // H
        return {
            "x": _w((lambda *s: _rng.normal(s) * 0.05)(B, S, D)),
            "wq": _w((lambda *s: _rng.normal(s) * 0.4)(D, H * Dh)),
            "wk": _w((lambda *s: _rng.normal(s) * 0.4)(D, Dh)),
            "wv": _w((lambda *s: _rng.normal(s) * 0.05)(D, Dh)),
            "wo": _w((lambda *s: _rng.normal(s) * 0.05)(H * Dh, D)),
        }
    _B_in = _B_setup()

    return {
        "A_x": _A_in["x"],
        "A_wqkv": _A_in["wqkv"],
        "A_wo": _A_in["wo"],
        "B_x": _B_in["x"],
        "B_wq": _B_in["wq"],
        "B_wk": _B_in["wk"],
        "B_wv": _B_in["wv"],
        "B_wo": _B_in["wo"],
    }

def reference(A_x, A_wqkv, A_wo, B_x, B_wq, B_wk, B_wv, B_wo):
    def _A_ref(x, wqkv, wo):
        B, S, D = x.shape
        H = 32; Dh = D // H
        qkv = (lambda x, *d: x.transpose(*d))((x @ wqkv).reshape(B, S, 3, H, Dh), 2, 0, 3, 1, 4)
        q, k, v = qkv[0], qkv[1], qkv[2]
        scale = Dh ** -0.5
        scores = jnp.einsum("bhqd,bhkd->bhqk", q, k) * scale
        p = _softmax(scores, axis=-1)
        o = jnp.einsum("bhqk,bhkd->bhqd", p, v)
        return (lambda x, *d: x.transpose(*d))(o, 0, 2, 1, 3).reshape(B, S, D) @ wo

    def _B_ref(x, wq, wk, wv, wo):
        B, S, D = x.shape
        H = 32
        Dh = D // H
        q = (lambda x, *d: x.transpose(*d))((x @ wq).reshape(B, S, H, Dh), 0, 2, 1, 3)
        k = x @ wk
        v = x @ wv
        scores = jnp.einsum("bhqd,bkd->bhqk", q, k) * (Dh ** -0.5)
        p = _softmax(scores, axis=-1)
        o = jnp.einsum("bhqk,bkd->bhqd", p, v)
        return (lambda x, *d: x.transpose(*d))(o, 0, 2, 1, 3).reshape(B, S, H * Dh) @ wo

    a = _A_ref(A_x, A_wqkv, A_wo)
    b = _B_ref(B_x, B_wq, B_wk, B_wv, B_wo)
    return jnp.concatenate([a, b], axis=-1)
```

```python
import functools
import math
import jax
import jax.numpy as jnp
from jax import lax
import jax.experimental.pallas as pl
import jax.experimental.pallas.tpu as pltpu

S = 2048
D = 640
H = 32
DH = 20
NG = 8
TK = 128
NC = S // TK
QB = 2
NQB = 16 // QB
NU = 2 * NG * NQB
W = 512 * QB
XC = 512
QSCALE = (DH ** -0.5) * math.log2(math.e)

_NT = (((1,), (1,)), ((), ()))
_TN = (((0,), (0,)), ((), ()))
F32 = jnp.float32
BF16 = jnp.bfloat16


def _kernel(ax, awqkv, awo, bx, bwq, bwk, bwv, bwo, out,
            lhs_a, wkt_a, lhs_b, wk4_b, kp, qt, vt, ot, s0, s1, m_ref):
    z = lambda r, c, dt: jnp.zeros((r, c), dt)
    lhs_b[0:D, :] = bwq[...].T
    wv = bwv[...].astype(F32)
    wv2 = jnp.concatenate([wv, z(D, 8, F32), wv, z(D, 80, F32)], axis=1)
    lhs_b[D:D + 48, :] = wv2.T[0:48, :].astype(BF16)
    wk = bwk[...].astype(F32)
    wk4_b[...] = jnp.concatenate([wk, z(D, 16, F32), wk, z(D, 16, F32), wk, z(D, 16, F32), wk], axis=1).astype(BF16)
    lhs_a[0:D, :] = awqkv[:, 0:D].T
    lhs_a[D:2 * D, :] = awqkv[:, 2 * D:3 * D].T
    wkt = awqkv[:, D:2 * D].astype(F32).T
    for g in range(NG):
        parts = []
        for v in range(4):
            r = 80 * g + 20 * v
            parts.append(wkt[r:r + 20, :])
            if v < 3:
                parts.append(z(16, D, F32))
        wkt_a[128 * g:128 * (g + 1), :] = jnp.concatenate(parts, axis=0).astype(BF16)

    row8 = lax.broadcasted_iota(jnp.int32, (8, XC), 0)
    lo4 = row8 < 4

    def proj_b(i, c):
        rows = pl.ds(pl.multiple_of(i * XC, XC), XC)
        xc = bx[rows, :]
        r = lax.dot_general(lhs_b[...], xc, _NT, preferred_element_type=F32)
        q = (r[0:D, :] * QSCALE).astype(BF16)
        vv = r[D:D + 48, :]
        vv = jnp.concatenate([vv[0:16], jnp.where(lo4, vv[16:24], 1.0), jnp.where(lo4, 1.0, vv[24:32]), vv[32:48]], axis=0)
        for j in range(XC // 128):
            qt[16 + i * (XC // 128) + j] = q[:, j * 128:(j + 1) * 128]
            vt[i * (XC // 128) + j, 768:816, :] = vv[:, j * 128:(j + 1) * 128]
        kp[NG, rows, :] = jnp.dot(xc, wk4_b[...], preferred_element_type=F32).astype(BF16)
        return c
    lax.fori_loop(0, S // XC, proj_b, 0)

    def proj_a(i, c):
        rows = pl.ds(pl.multiple_of(i * XC, XC), XC)
        xc = ax[rows, :]
        r = lax.dot_general(lhs_a[...], xc, _NT, preferred_element_type=F32)
        q = (r[0:D, :] * QSCALE).astype(BF16)
        parts = []
        for p in range(16):
            b = D + 40 * p
            mid = r[b + 16:b + 24]
            parts += [r[b:b + 16], jnp.where(lo4, mid, 1.0), jnp.where(lo4, 1.0, mid), r[b + 24:b + 40]]
        vv = jnp.concatenate(parts, axis=0)
        for j in range(XC // 128):
            qt[i * (XC // 128) + j] = q[:, j * 128:(j + 1) * 128]
            vt[i * (XC // 128) + j, 0:768, :] = vv[:, j * 128:(j + 1) * 128]
        k = lax.dot_general(xc, wkt_a[...], _NT, preferred_element_type=F32).astype(BF16)
        for g in range(NG):
            kp[g, rows, :] = k[:, 128 * g:128 * (g + 1)]
        return c
    lax.fori_loop(0, S // XC, proj_a, 0)

    def decode(u):
        br = u // (NG * NQB)
        r = u % (NG * NQB)
        return br, r // NQB, r % NQB

    def step(u_next, u_cur, s_next, s_cur):
        do1 = u_next is not None
        do2 = u_cur is not None
        if do1:
            br_n, g_n, qb_n = decode(u_next)
            kidx = jnp.where(br_n == 0, g_n, NG)
            r0 = pl.multiple_of(g_n * 80, 16)
        if do2:
            br_c, g_c, qb_c = decode(u_cur)
            vrow = [pl.multiple_of(jnp.where(br_c == 0, 96 * g_c + 24 * v, 768 + 24 * (v % 2)), 8) for v in range(4)]
            m_cur = m_ref[...]
        ms = []
        for j in range(QB):
            lanes = slice(j * 512, (j + 1) * 512)
            if do1:
                zz = jnp.zeros((32, 128), BF16)
                cols = []
                for v in range(4):
                    qblk = qt[br_n * 16 + qb_n * QB + j, pl.ds(r0 + 16 * v, 32), :]
                    cols.append(jnp.concatenate([zz] * v + [qblk] + [zz] * (3 - v), axis=0))
                w = jnp.concatenate(cols, axis=1)
                mx = None
            if do2:
                acc = [None] * 4
            for c in range(NC):
                rows = pl.ds(c * TK, TK)
                if do1:
                    s = jnp.dot(kp[kidx, rows, :], w, preferred_element_type=F32)
                    s_next[rows, lanes] = s
                    mc = jnp.max(s.reshape(TK // 8, 8, 512), axis=0)
                    mx = mc if mx is None else jnp.maximum(mx, mc)
                if do2:
                    for v in range(4):
                        ls = slice(j * 512 + v * 128, j * 512 + (v + 1) * 128)
                        p = jnp.exp2(s_cur[rows, ls] - m_cur[:, ls])
                        d = jnp.dot(vt[c, pl.ds(vrow[v], 24), :], p, preferred_element_type=F32,
                                    precision=lax.Precision.DEFAULT)
                        acc[v] = d if acc[v] is None else acc[v] + d
            if do2:
                outs = []
                for v in range(4):
                    lrow = 23 if v % 2 == 0 else 0
                    o = 0 if v % 2 == 0 else 4
                    l = acc[v][lrow:lrow + 1, :]
                    outs.append((acc[v] * (1.0 / l))[o:o + 20])
                ot[br_c * 16 + qb_c * QB + j, pl.ds(pl.multiple_of(g_c * 80, 16), 80), :] = (
                    jnp.concatenate(outs, axis=0).astype(BF16))
            if do1:
                ms.append(jnp.max(mx, axis=0, keepdims=True))
        if do1:
            m_ref[...] = jnp.concatenate(ms, axis=1) if QB > 1 else ms[0]

    step(0, None, s0, None)

    def body(u, c):
        @pl.when(u % 2 == 0)
        def _():
            step(u + 1, u, s1, s0)

        @pl.when(u % 2 == 1)
        def _():
            step(u + 1, u, s0, s1)
        return c
    lax.fori_loop(0, NU - 1, body, 0)
    step(None, NU - 1, None, s1)

    for br, wo in ((0, awo), (1, bwo)):
        def oproj(i, c, br=br, wo=wo):
            o_t = jnp.concatenate([ot[br * 16 + i * 4 + j] for j in range(4)], axis=1)
            res = lax.dot_general(o_t, wo[...], _TN, preferred_element_type=F32)
            out[pl.ds(pl.multiple_of(i * 512, 512), 512), br * D:(br + 1) * D] = res.astype(BF16)
            return c
        lax.fori_loop(0, 4, oproj, 0)


@jax.jit
def pallas_concat_heads__softmax_full_mha__grouped_kv_mqa__prompt_kernel(
    A_x, A_wqkv, A_wo, B_x, B_wq, B_wk, B_wv, B_wo,
):
    out = pl.pallas_call(
        _kernel,
        out_shape=jax.ShapeDtypeStruct((S, 2 * D), BF16),
        scratch_shapes=[
            pltpu.VMEM((2 * D, D), BF16),
            pltpu.VMEM((1024, D), BF16),
            pltpu.VMEM((D + 48, D), BF16),
            pltpu.VMEM((D, 128), BF16),
            pltpu.VMEM((NG + 1, S, 128), BF16),
            pltpu.VMEM((32, D, 128), BF16),
            pltpu.VMEM((NC, 816, 128), F32),
            pltpu.VMEM((32, D, 128), BF16),
            pltpu.VMEM((S, W), F32),
            pltpu.VMEM((S, W), F32),
            pltpu.VMEM((1, W), F32),
        ],
        compiler_params=pltpu.CompilerParams(vmem_limit_bytes=100 * 1024 * 1024),
        name="mha_mqa",
    )(A_x.reshape(S, D), A_wqkv, A_wo, B_x.reshape(S, D), B_wq, B_wk, B_wv, B_wo)
    return out.reshape(1, S, 2 * D)
```

```python
import math
import jax
import jax.numpy as jnp
from jax import lax
import jax.experimental.pallas as pl
import jax.experimental.pallas.tpu as pltpu

S = 2048
D = 640
DH = 20
NG = 8
TK = 128
NC = S // TK
NQB = 16
NU = 2 * NG * NQB
NH = 12
ORDER = 2
LAGS = (1, 1, 1, 1)
NPRE = (NU - 1) % NH
XC = 512
NXC = S // XC
OC = 256
NOC = S // OC
QSCALE = (DH ** -0.5) * math.log2(math.e)

_NT = (((1,), (1,)), ((), ()))
_TN = (((0,), (0,)), ((), ()))
F32 = jnp.float32
BF16 = jnp.bfloat16


def _kernel(ax_h, awqkv_h, awo_h, bx_h, bwq_h, bwkt_h, bwvt_h, bwo_h, out_h,
            ax, awqkv, awo, bx, bwq, bwkt, bwvt, bwo, outv,
            lhs_a, lhs_b, wk_b, kp, qt, vt, ot, zero_ref, sem, osem, *sbufs):
    bufs = (sbufs[:NC], sbufs[NC:])

    def cp(src, dst, k):
        return pltpu.make_async_copy(src, dst, sem.at[k])

    def xrows(i):
        return pl.ds(i * XC, XC)

    c_bwq = cp(bwq_h, bwq, 0)
    c_bwk = cp(bwkt_h, bwkt, 1)
    c_bwv = cp(bwvt_h, bwvt, 2)
    c_bx = [cp(bx_h.at[xrows(i)], bx.at[xrows(i)], 3 + i) for i in range(NXC)]
    c_awqkv = cp(awqkv_h, awqkv, 7)
    c_ax = [cp(ax_h.at[xrows(i)], ax.at[xrows(i)], 8 + i) for i in range(NXC)]
    c_awo = cp(awo_h, awo, 12)
    c_bwo = cp(bwo_h, bwo, 13)

    c_bwq.start()
    c_bwk.start()
    c_bwv.start()
    c_bx[0].start()
    zero_ref[0] = 0

    z = lambda r, c, dt: jnp.zeros((r, c), dt)
    lo4 = lax.broadcasted_iota(jnp.int32, (8, XC), 0) < 4

    c_bwq.wait()
    c_bwk.wait()
    c_bwv.wait()
    for i in range(1, NXC):
        c_bx[i].start()
    c_awqkv.start()
    lhs_b[0:D, :] = bwq[...].T
    wv = bwvt[...].astype(F32)
    lhs_b[D:D + 48, :] = jnp.concatenate([wv, z(8, D, F32), wv], axis=0).astype(BF16)
    wk = bwkt[...].astype(F32)
    wk_b[...] = jnp.concatenate([wk, wk, wk, wk, z(48, D, F32)], axis=0).T.astype(BF16)

    def prep_a():
        lhs_a[0:D, :] = awqkv[:, 0:D].T
        lhs_a[D:2 * D, :] = awqkv[:, 2 * D:3 * D].T

    def store_q(r, qb0):
        q = r * QSCALE
        z8 = z(8, XC, F32)
        for g in range(NG):
            t = [q[80 * g + 8 * k:80 * g + 8 * (k + 1)] for k in range(10)]
            blk = jnp.concatenate(
                [t[0], t[1], jnp.where(lo4, t[2], 0.0), z8,
                 jnp.where(lo4, 0.0, t[2]), t[3], t[4], z8,
                 z8, t[5], t[6], jnp.where(lo4, t[7], 0.0),
                 z8, jnp.where(lo4, 0.0, t[7]), t[8], t[9]], axis=0).astype(BF16)
            for j in range(XC // 128):
                qt[(qb0 + j) * NG + g] = blk[:, j * 128:(j + 1) * 128]

    def v_pair(r, b):
        mid = r[b + 16:b + 24]
        return [r[b:b + 16], jnp.where(lo4, mid, 1.0), jnp.where(lo4, 1.0, mid), r[b + 24:b + 40]]

    def proj_b(i):
        xc = bx[xrows(i), :]
        r = lax.dot_general(lhs_b[...], xc, _NT, preferred_element_type=F32)
        store_q(r[0:D], 16 + i * (XC // 128))
        vv = jnp.concatenate([r[D:D + 16], jnp.where(lo4, r[D + 16:D + 24], 1.0),
                              jnp.where(lo4, 1.0, r[D + 24:D + 32]), r[D + 32:D + 48]], axis=0)
        for j in range(XC // 128):
            vt[NG, i * (XC // 128) + j, 0:48, :] = vv[:, j * 128:(j + 1) * 128]
            vt[NG, i * (XC // 128) + j, 48:96, :] = vv[:, j * 128:(j + 1) * 128]
            kp[NG, pl.ds(i * XC + j * 128, 128), :] = jnp.dot(
                xc[j * 128:(j + 1) * 128], wk_b[...], preferred_element_type=F32).astype(BF16)

    for i in range(NXC):
        c_bx[i].wait()
        if i == 0:
            for k in range(NXC):
                c_ax[k].start()
        if i == NXC - 1:
            c_awqkv.wait()
            c_awo.start()
            c_bwo.start()
            prep_a()
        proj_b(i)

    for k in range(NXC):
        c_ax[k].wait()

    def proj_a(i, c):
        rows = pl.ds(pl.multiple_of(i * XC, XC), XC)
        xc = ax[rows, :]
        for j in range(XC // 128):
            k = jnp.dot(xc[j * 128:(j + 1) * 128], awqkv[:, D:2 * D], preferred_element_type=F32).astype(BF16)
            k = jnp.concatenate([k, z(128, 128, BF16)], axis=1)
            for g in range(NG):
                kp[g, pl.ds(pl.multiple_of(i * XC + j * 128, 128), 128), :] = k[:, 80 * g:80 * g + 128]
        r = lax.dot_general(lhs_a[...], xc, _NT, preferred_element_type=F32)
        store_q(r[0:D], i * (XC // 128))
        for g in range(NG):
            vv = jnp.concatenate(v_pair(r, D + 80 * g) + v_pair(r, D + 80 * g + 40), axis=0)
            for j in range(XC // 128):
                vt[g, i * (XC // 128) + j] = vv[:, j * 128:(j + 1) * 128]
        return c
    lax.fori_loop(0, NXC, proj_a, 0)

    def decode(u):
        br = u // (NG * NQB)
        r = u % (NG * NQB)
        return br, r // NQB, r % NQB

    class P1:
        def __init__(self, u, buf):
            br, g, qb = decode(u)
            self.kidx = jnp.where(br == 0, g, NG)
            qm = qt[(br * 16 + qb) * NG + g]
            self.w = []
            for v in range(4):
                parts = [qm[32 * v:32 * (v + 1)], z(96 - 16 * v, 128, BF16)]
                if v:
                    parts = [z(16 * v, 128, BF16)] + parts
                self.w.append(jnp.concatenate(parts, axis=0))
            self.mx = [None] * 4
            self.buf = buf

        def chunk(self, c, v):
            s = jnp.dot(kp[self.kidx, pl.ds(c * TK, TK), :], self.w[v], preferred_element_type=F32)
            self.buf[c][0, :, v * 128:(v + 1) * 128] = s
            mc = jnp.max(s.reshape(TK // 8, 8, 128), axis=0)
            self.mx[v] = mc if self.mx[v] is None else jnp.maximum(self.mx[v], mc)

        def finish(self, v):
            return jnp.max(self.mx[v], axis=0, keepdims=True)

    class P2:
        def __init__(self, u, buf, zoff):
            self.br, self.g, self.qb = decode(u)
            self.vidx = jnp.where(self.br == 0, self.g, NG)
            self.acc = [None] * 4
            self.buf, self.zoff = buf, zoff
            self.ndone = 0

        def chunk(self, c, v, m):
            ls = slice(v * 128, (v + 1) * 128)
            p = jnp.exp2(self.buf[c][self.zoff, :, ls] - m)
            d = jnp.dot(vt[self.vidx, c, 24 * v:24 * (v + 1), :], p, preferred_element_type=F32,
                        precision=lax.Precision.DEFAULT)
            self.acc[v] = d if self.acc[v] is None else self.acc[v] + d
            if c == NC - 1:
                self.ndone += 1
                if self.ndone == 4:
                    self.finish()

        def finish(self):
            outs = []
            for v in range(4):
                lrow = 23 if v % 2 == 0 else 0
                o = 0 if v % 2 == 0 else 4
                l = self.acc[v][lrow:lrow + 1, :]
                outs.append((self.acc[v] * (1.0 / l))[o:o + 20])
            ot[self.br * 16 + self.qb, pl.ds(pl.multiple_of(self.g * 80, 16), 80), :] = (
                jnp.concatenate(outs, axis=0).astype(BF16))

    def run(u0, par0, n1, n2, m, zoff, extra=()):
        ms = {}
        if m is not None:
            for v in range(4):
                ms[(0, v)] = m[:, v * 128:(v + 1) * 128]
        p1s, p2s = {}, {}
        lags = LAGS if n1 else (0, 0, 0, 0)
        extra = list(extra)

        def do1(k, v):
            if k < n1 * NC:
                t, c = divmod(k, NC)
                if t not in p1s:
                    p1s[t] = P1(u0 + t + 1, bufs[(par0 + t + 1) % 2])
                p1s[t].chunk(c, v)
                if c == NC - 1:
                    ms[(t + 1, v)] = p1s[t].finish(v)

        def do2(k, v):
            k2 = k - lags[v]
            if 0 <= k2 < n2 * NC:
                t, c = divmod(k2, NC)
                if t not in p2s:
                    p2s[t] = P2(u0 + t, bufs[(par0 + t) % 2], zoff)
                p2s[t].chunk(c, v, ms[(t, v)])

        for k in range(max(n1 * NC, n2 * NC + max(lags))):
            if ORDER == 0:
                for v in range(4):
                    do1(k, v)
                for v in range(4):
                    do2(k, v)
            elif ORDER == 1:
                for v in range(4):
                    do1(k, v)
                    do2(k, v)
            elif ORDER == 2:
                for v in range(4):
                    do1(k, v)
                    do2(k, (v + 2) % 4)
            if extra:
                extra.pop(0)()
        for f in extra:
            f()
        if n1:
            return jnp.concatenate([ms[(n1, v)] for v in range(4)], axis=1)

    zoff0 = zero_ref[0]
    m0 = run(-1, 1, 1, 0, None, None)
    if NPRE:
        m0 = run(0, 0, NPRE, NPRE, m0, zoff0)

    def body(i, m):
        return run(NPRE + i * NH, NPRE % 2, NH, NH, m, zero_ref[0])
    m_last = lax.fori_loop(0, (NU - 1 - NPRE) // NH, body, m0)

    c_awo.wait()
    c_bwo.wait()

    def ocopy(i):
        rows = pl.ds(i * OC, OC)
        return pltpu.make_async_copy(outv.at[rows], out_h.at[rows], osem.at[i])

    def oproj(i):
        rows = pl.ds(i * OC, OC)
        for br, wo in ((0, awo), (1, bwo)):
            o_t = jnp.concatenate([ot[br * 16 + i * (OC // 128) + j] for j in range(OC // 128)], axis=1)
            res = lax.dot_general(o_t, wo[...], _TN, preferred_element_type=F32)
            outv[rows, br * D:(br + 1) * D] = res.astype(BF16)
        ocopy(i).start()

    pieces = []
    for br, wo in ((0, awo), (1, bwo)):
        for j in range(OC // 128):
            o_n = ot[br * 16 + j].T
            for n in range(D // 128):
                def piece(br=br, wo=wo, j=j, n=n, o_n=o_n):
                    res = jnp.dot(o_n, wo[:, n * 128:(n + 1) * 128], preferred_element_type=F32)
                    outv[j * 128:(j + 1) * 128, br * D + n * 128:br * D + (n + 1) * 128] = res.astype(BF16)
                pieces.append(piece)
    run(NU - 1, (NU - 1) % 2, 0, 1, m_last, 0, extra=pieces)
    ocopy(0).start()
    for i in range(1, NOC):
        oproj(i)
    for i in range(NOC):
        ocopy(i).wait()


@jax.jit
def pallas_concat_heads__softmax_full_mha__grouped_kv_mqa__prompt_kernel(
    A_x, A_wqkv, A_wo, B_x, B_wq, B_wk, B_wv, B_wo,
):
    anyspec = pl.BlockSpec(memory_space=pl.ANY)
    out = pl.pallas_call(
        _kernel,
        out_shape=jax.ShapeDtypeStruct((S, 2 * D), BF16),
        in_specs=[anyspec] * 8,
        out_specs=anyspec,
        scratch_shapes=[
            pltpu.VMEM((S, D), BF16),
            pltpu.VMEM((D, 3 * D), BF16),
            pltpu.VMEM((D, D), BF16),
            pltpu.VMEM((S, D), BF16),
            pltpu.VMEM((D, D), BF16),
            pltpu.VMEM((DH, D), BF16),
            pltpu.VMEM((DH, D), BF16),
            pltpu.VMEM((D, D), BF16),
            pltpu.VMEM((S, 2 * D), BF16),
            pltpu.VMEM((2 * D, D), BF16),
            pltpu.VMEM((D + 48, D), BF16),
            pltpu.VMEM((D, 128), BF16),
            pltpu.VMEM((NG + 1, S, 128), BF16),
            pltpu.VMEM((32 * NG, 128, 128), BF16),
            pltpu.VMEM((NG + 1, NC, 96, 128), F32),
            pltpu.VMEM((32, D, 128), BF16),
            pltpu.SMEM((1,), jnp.int32),
            pltpu.SemaphoreType.DMA((14,)),
            pltpu.SemaphoreType.DMA((NOC,)),
        ] + [pltpu.VMEM((1, TK, 512), F32)] * (2 * NC),
        compiler_params=pltpu.CompilerParams(vmem_limit_bytes=100 * 1024 * 1024),
        name="mha_mqa",
    )(A_x.reshape(S, D), A_wqkv, A_wo, B_x.reshape(S, D), B_wq, B_wk.T, B_wv.T, B_wo)
    return out.reshape(1, S, 2 * D)
```

```python
import math
import jax
import jax.numpy as jnp
from jax import lax
import jax.experimental.pallas as pl
import jax.experimental.pallas.tpu as pltpu

S = 2048
D = 640
H = 32
DH = 20
TK = 128
NC = S // TK
NQB = 16
NU = 2 * H * 4
NH = 12
NPRE = 3
XC = 512
NXC = S // XC
OC = 256
NOC = S // OC
QSCALE = (DH ** -0.5) * math.log2(math.e)

X = 10
NV = 16 * X
NM = S - NV
PK = 5
DS = 5
T0 = -200
T1 = 250
TS = 150
GD = 300
NPG = 2
PGD = 500
LAG = 3
_g16 = NM // 16
MSZ = [16 * (_g16 // NC + (1 if c < _g16 % NC else 0)) for c in range(NC)]
MOFF = [NV + sum(MSZ[:c]) for c in range(NC)]
NR = -(-(NV // 8) // PK)
SLOT = 24 + NM // NC

_NT = (((1,), (1,)), ((), ()))
_TN = (((0,), (0,)), ((), ()))
F32 = jnp.float32
BF16 = jnp.bfloat16


def _kernel(ax_h, awqkv_h, awo_h, bx_h, bwq_h, bwkt_h, bwvt_h, bwo_h, out_h,
            ax, awqkv, awo, bx, bwq, bwo, outv,
            lhs_a, lhs_b, wk_b, kp, qt, vt, ot, kb0, kb1, kb2, zero_ref, sem, osem, *rest):
    qss = (rest[0:4], rest[4:8])
    rest = rest[8:]
    sbufs, (bwkt, bwvt) = rest[:2 * NC], rest[2 * NC:2 * NC + 2]
    bufs = (sbufs[:NC], sbufs[NC:])
    kbs = (kb0, kb1, kb2)

    def cp(src, dst, k):
        return pltpu.make_async_copy(src, dst, sem.at[k])

    def xrows(i):
        return pl.ds(i * XC, XC)

    c_bwq = cp(bwq_h, bwq, 0)
    c_bwk = cp(bwkt_h, bwkt, 1)
    c_bwv = cp(bwvt_h, bwvt, 2)
    c_bx = [cp(bx_h.at[xrows(i)], bx.at[xrows(i)], 3 + i) for i in range(NXC)]
    c_awqkv = cp(awqkv_h, awqkv, 7)
    c_ax = [cp(ax_h.at[xrows(i)], ax.at[xrows(i)], 8 + i) for i in range(NXC)]
    c_awo = cp(awo_h, awo, 12)
    c_bwo = cp(bwo_h, bwo, 13)

    c_bwq.start()
    c_bwk.start()
    c_bwv.start()
    c_bx[0].start()
    zero_ref[0] = 0
    for padr in rest[2 * NC + 2:]:
        padr[...] = jnp.zeros((8, 128), F32)

    z = lambda r, c, dt: jnp.zeros((r, c), dt)

    c_bwq.wait()
    c_bwk.wait()
    c_bwv.wait()
    for i in range(1, NXC):
        c_bx[i].start()
    c_awqkv.start()
    lhs_b[0:D, :] = bwq[...].T
    wv = bwvt[...].astype(F32)
    lhs_b[D:D + 32, :] = jnp.concatenate([wv, z(12, D, F32)], axis=0).astype(BF16)
    wk = bwkt[...].astype(F32)
    wk_b[...] = jnp.concatenate([wk, z(108, D, F32)], axis=0).T.astype(BF16)

    def prep_a():
        lhs_a[0:D, :] = awqkv[:, 0:D].T
        lhs_a[D:2 * D, :] = awqkv[:, 2 * D:3 * D].T

    def store_q(r, br, qb0):
        q = r * QSCALE
        for h in range(H):
            blk = jnp.concatenate([q[DH * h:DH * (h + 1)], z(12, XC, F32)], axis=0).astype(BF16)
            blk = pltpu.bitcast(blk, F32)
            for j in range(XC // 128):
                qt[(br * H + h) * NQB + qb0 + j] = blk[:, j * 128:(j + 1) * 128]

    def store_v(rows20, hidx, c0):
        vv = jnp.concatenate([rows20, jnp.ones((4, XC), F32)], axis=0)
        for j in range(XC // 128):
            vt[hidx, c0 + j, 0:24, :] = vv[:, j * 128:(j + 1) * 128]

    def proj_b(i):
        xc = bx[xrows(i), :]
        r = lax.dot_general(lhs_b[0:D + 32, :], xc, _NT, preferred_element_type=F32)
        store_q(r[0:D], 1, i * (XC // 128))
        store_v(r[D:D + DH], H, i * (XC // 128))
        for j in range(XC // 128):
            k = jnp.dot(xc[j * 128:(j + 1) * 128], wk_b[...], preferred_element_type=F32).astype(BF16)
            kp[H, pl.ds(i * (XC // 2) + j * 64, 64), :] = pltpu.bitcast(k, F32)

    for i in range(NXC):
        c_bx[i].wait()
        if i == 0:
            for k in range(NXC):
                c_ax[k].start()
        if i == NXC - 1:
            c_awqkv.wait()
            c_awo.start()
            c_bwo.start()
            prep_a()
        proj_b(i)

    for k in range(NXC):
        c_ax[k].wait()

    lane = lax.broadcasted_iota(jnp.int32, (64, 128), 1)

    def proj_a(i, c):
        rows = pl.ds(pl.multiple_of(i * XC, XC), XC)
        xc = ax[rows, :]
        for j in range(XC // 128):
            k = jnp.dot(xc[j * 128:(j + 1) * 128], awqkv[:, D:2 * D], preferred_element_type=F32).astype(BF16)
            k = pltpu.bitcast(k, F32)
            for h in range(H):
                t, off = divmod(DH * h, 128)
                win = k[:, 128 * t:128 * (t + 1)]
                if off:
                    win = pltpu.roll(win, 128 - off, 1)
                if off + DH > 128:
                    nxt = pltpu.roll(k[:, 128 * (t + 1):128 * (t + 2)], 128 - off, 1)
                    win = jnp.where(lane < 128 - off, win, nxt)
                kp[h, pl.ds(pl.multiple_of(i * (XC // 2) + j * 64, 64), 64), :] = win
        r = lax.dot_general(lhs_a[...], xc, _NT, preferred_element_type=F32)
        store_q(r[0:D], 0, i * (XC // 128))
        for h in range(H):
            store_v(r[D + DH * h:D + DH * (h + 1)], h, i * (XC // 128))
        return c
    lax.fori_loop(0, NXC, proj_a, 0)

    def st(buf, r0, n, v, val):
        o = 0
        while o < n:
            c, rr = divmod(r0 + o, TK)
            k = min(n - o, TK - rr)
            buf[c][0, rr:rr + k, v * 128:(v + 1) * 128] = val[o:o + k]
            o += k

    def produce(kidx, kb, g, d0, d1, flag, gate):
        k32 = kp[kidx, 8 * g:8 * (g + 1), :]
        if gate is not None:
            k32 = jnp.where(flag, gate, k32)
        kf = pltpu.bitcast(k32, BF16).astype(F32)
        for d in range(d0, d1):
            bc = jnp.broadcast_to(kf[:, d:d + 1], (16, 128))
            for r in range(2):
                pr, a = divmod(2 * g + r, PK)
                kb[0, pr * DH + d, 8 * a:8 * (a + 1), :] = bc[8 * r:8 * (r + 1)]

    class P1:
        def __init__(self, u, s, off):
            bh = u // 4
            self.bh = bh
            self.kidx = jnp.minimum(bh, H)
            self.qc = qc = s % 4
            self.hs = s // 4
            self.off = off and X > 0
            self.msz = MSZ if self.off else [TK] * NC
            self.moff = MOFF if self.off else [TK * c for c in range(NC)]
            self.qblk = [pltpu.bitcast(qt[bh * NQB + qc * 4 + v], BF16) for v in range(4)]
            self.w = [jnp.concatenate([b, z(96, 128, BF16)], axis=0) for b in self.qblk]
            self.mx = [None] * 4
            self.mv = [None] * 4
            self.buf = bufs[s % 2]
            self.qs = qss[s % 2]

        def upd(self, v, val):
            self.mx[v] = val if self.mx[v] is None else jnp.maximum(self.mx[v], val)

        def build(self, v, zoff, flag, gate):
            kb = kbs[self.hs % 3]
            qs = self.qs[v]
            qf = self.qblk[v].astype(F32)
            for d in range(DH):
                row = jnp.broadcast_to(qf[d:d + 1], (8, 128))
                if d == 0 and gate is not None:
                    row = jnp.where(flag, gate, row)
                qs[0, d] = row
            vals = []
            for r in range(NR):
                n = min(PK, NV // 8 - r * PK)
                acc = None
                for d in range(DH):
                    t = kb[zoff, r * DH + d, 0:8 * n, :].reshape(n, 8, 128) * qs[zoff, d][None]
                    acc = t if acc is None else acc + t
                    if (d + 1) % DS == 0:
                        vals += [acc[j] for j in range(n)]
                st(self.buf, r * PK * 8, 8 * n, v, acc.reshape(8 * n, 128))
                am = jnp.max(acc, axis=0)
                self.mv[v] = am if self.mv[v] is None else jnp.maximum(self.mv[v], am)
            return vals

        def chunk(self, c, v, flag, anch):
            kc = kp[self.kidx, pl.ds(self.moff[c] // 2, self.msz[c] // 2), :]
            if anch:
                parts = []
                for j in range(self.msz[c] // 16):
                    p32 = kc[8 * j:8 * (j + 1)]
                    for val in anch.get(j, []):
                        p32 = jnp.where(flag, val, p32)
                    parts.append(p32)
                kc = jnp.concatenate(parts, axis=0)
            s = jnp.dot(pltpu.bitcast(kc, BF16), self.w[v], preferred_element_type=F32)
            st(self.buf, self.moff[c], self.msz[c], v, s)
            self.upd(v, jnp.max(s.reshape(self.msz[c] // 8, 8, 128), axis=0))
            return s[0:8]

        def finish(self, v):
            m = jnp.maximum(self.mx[v], self.mv[v]) if self.off else self.mx[v]
            return jnp.max(m, axis=0, keepdims=True)

    class P2:
        def __init__(self, u, qc, par, zoff):
            self.bh = u // 4
            self.qc = qc
            self.vidx = jnp.minimum(self.bh, H)
            self.acc = [None] * 4
            self.buf, self.zoff = bufs[par], zoff

        def chunk(self, c, v, m):
            p = jnp.exp2(self.buf[c][self.zoff, :, v * 128:(v + 1) * 128] - m)
            d = jnp.dot(vt[self.vidx, c, 0:24, :], p, preferred_element_type=F32,
                        precision=lax.Precision.DEFAULT)
            self.acc[v] = d if self.acc[v] is None else self.acc[v] + d
            if c == NC - 1:
                a = self.acc[v]
                br, h = self.bh // H, self.bh % H
                ot[br * NQB + self.qc * 4 + v, pl.ds(pl.multiple_of(h * 24, 8), 24), :] = a * (1.0 / a[23:24, :])

    def run(u0, s0, n1, n2, m, zoff, extra=()):
        ms = {}
        if m is not None:
            for v in range(4):
                ms[(0, v)] = m[:, v * 128:(v + 1) * 128]
        p1s, p2s = {}, {}
        lag = LAG if n1 else 0
        extra = list(extra)
        flag = (jnp.full((8, 128), zoff, jnp.int32) != 0) if n1 else None

        def getp1(t):
            if t not in p1s:
                p1s[t] = P1(u0 + t + 1, s0 + t + 1, s0 + t + 1 > 0)
            return p1s[t]

        njobs = n1 * NC * 4
        jt = lambda n: n * SLOT // 4
        nj = lambda n: (MSZ if s0 + n // (4 * NC) + 1 > 0 else [TK] * NC)[(n // 4) % NC] // 16
        pts = sorted((jt(n) + 16 * j, n, j) for n in range(njobs) for j in range(nj(n)))
        builds = {}
        anchors = {}
        gates = {}
        L = SLOT * NC
        per_col = sum(min(PK, NV // 8 - r * PK) for r in range(NR)) * (DH // DS)
        for t in range(n1):
            if not X:
                break
            if s0 + t + 1 > 0:
                w = [p for p in pts if max(t * L + T0, TS) <= p[0] <= (t + 1) * L - T1]
                for v in range(4):
                    mine = [w[(v * per_col + i) * len(w) // (4 * per_col)] for i in range(per_col)]
                    first = min(p[1] for p in mine)
                    gj = max([n for n in range(first) if jt(n) <= mine[0][0] - GD], default=None)

                    def bld(t=t, v=v, mine=mine, gj=gj):
                        vals = getp1(t).build(v, zoff, flag, None if gj is None else gates[gj])
                        for val, p in zip(vals, mine):
                            anchors.setdefault(p[1], {}).setdefault(p[2], []).append(val)
                    builds.setdefault(first, []).append(bld)
            s = s0 + t + 1
            grp = [(s // 4 + 1, g, k) for g in range(X * (s % 4) // 4, X * (s % 4 + 1) // 4) for k in range(NPG)]
            if s == 0:
                grp = [(0, g, k) for g in range(X) for k in range(NPG)] + grp
            w = [p for p in pts if max(t * L, TS + 100) <= p[0] <= (t + 1) * L - 300]
            for i, (hs, g, k) in enumerate(grp):
                p = w[(2 * i + 1) * len(w) // (2 * len(grp))]

                gj = max([n for n in range(p[1]) if jt(n) <= p[0] - PGD], default=None)

                def prod(t=t, hs=hs, g=g, k=k, p=p, s=s, gj=gj):
                    kidx = jnp.minimum(getp1(t).bh + (hs - s // 4), H)
                    produce(kidx, kbs[hs % 3], g, DH * k // NPG, DH * (k + 1) // NPG,
                            flag, None if gj is None else gates[gj])
                    pr, a = divmod(2 * g, PK)
                    val = kbs[hs % 3][zoff, pr * DH + DH * k // NPG, 8 * a:8 * (a + 1), :]
                    anchors.setdefault(p[1], {}).setdefault(p[2], []).append(val)
                builds.setdefault(p[1], []).append(prod)

        for k in range(max(n1 * NC, n2 * NC + lag)):
            for vi in range(4):
                if k < n1 * NC:
                    t, c = divmod(k, NC)
                    n = 4 * k + vi
                    for f in builds.get(n, []):
                        f()
                    gates[n] = getp1(t).chunk(c, vi, flag, anchors.get(n))
                    if c == NC - 1:
                        ms[(t + 1, vi)] = p1s[t].finish(vi)
                k2 = k - lag
                v = (vi + 2) % 4
                if 0 <= k2 < n2 * NC:
                    t, c = divmod(k2, NC)
                    if t not in p2s:
                        p2s[t] = P2(u0 + t, (s0 + t) % 4, (s0 + t) % 2, zoff)
                    p2s[t].chunk(c, v, ms[(t, v)])
            if extra:
                extra.pop(0)()
        for f in extra:
            f()
        if n1:
            return jnp.concatenate([ms[(n1, v)] for v in range(4)], axis=1)

    zoff0 = zero_ref[0]
    m0 = run(-1, -1, 1, 0, None, zoff0)
    m0 = run(0, 0, NPRE, NPRE, m0, zoff0)

    def body(i, m):
        return run(NPRE + i * NH, NPRE, NH, NH, m, zero_ref[0])
    m_last = lax.fori_loop(0, (NU - 1 - NPRE) // NH, body, m0)

    c_awo.wait()
    c_bwo.wait()

    def ocopy(i):
        rows = pl.ds(i * OC, OC)
        return pltpu.make_async_copy(outv.at[rows], out_h.at[rows], osem.at[i])

    def o_t(br, qb):
        o24 = ot[br * NQB + qb]
        return jnp.concatenate([o24[24 * h:24 * h + DH] for h in range(H)], axis=0).astype(BF16)

    def oproj(i):
        rows = pl.ds(i * OC, OC)
        for br, wo in ((0, awo), (1, bwo)):
            o = jnp.concatenate([o_t(br, i * (OC // 128) + j) for j in range(OC // 128)], axis=1)
            res = lax.dot_general(o, wo[...], _TN, preferred_element_type=F32)
            outv[rows, br * D:(br + 1) * D] = res.astype(BF16)
        ocopy(i).start()

    pieces = []
    for br, wo in ((0, awo), (1, bwo)):
        for j in range(OC // 128):
            o_n = o_t(br, j).T
            for n in range(D // 128):
                def piece(br=br, wo=wo, j=j, n=n, o_n=o_n):
                    res = jnp.dot(o_n, wo[:, n * 128:(n + 1) * 128], preferred_element_type=F32)
                    outv[j * 128:(j + 1) * 128, br * D + n * 128:br * D + (n + 1) * 128] = res.astype(BF16)
                pieces.append(piece)
    run(NU - 1, 3, 0, 1, m_last, 0, extra=pieces)
    ocopy(0).start()
    for i in range(1, NOC):
        oproj(i)
    for i in range(NOC):
        ocopy(i).wait()


@jax.jit
def pallas_concat_heads__softmax_full_mha__grouped_kv_mqa__prompt_kernel(
    A_x, A_wqkv, A_wo, B_x, B_wq, B_wk, B_wv, B_wo,
):
    anyspec = pl.BlockSpec(memory_space=pl.ANY)
    out = pl.pallas_call(
        _kernel,
        out_shape=jax.ShapeDtypeStruct((S, 2 * D), BF16),
        in_specs=[anyspec] * 8,
        out_specs=anyspec,
        scratch_shapes=[
            pltpu.VMEM((S, D), BF16),
            pltpu.VMEM((D, 3 * D), BF16),
            pltpu.VMEM((D, D), BF16),
            pltpu.VMEM((S, D), BF16),
            pltpu.VMEM((D, D), BF16),
            pltpu.VMEM((D, D), BF16),
            pltpu.VMEM((S, 2 * D), BF16),
            pltpu.VMEM((2 * D, D), BF16),
            pltpu.VMEM((D + 64, D), BF16),
            pltpu.VMEM((D, 128), BF16),
            pltpu.VMEM((H + 1, S // 2, 128), F32),
            pltpu.VMEM((2 * H * NQB, 16, 128), F32),
            pltpu.VMEM((H + 1, NC, 32, 128), F32),
            pltpu.VMEM((2 * NQB, H * 24, 128), F32),
            pltpu.VMEM((1, max(NR, 1) * DH, 8 * PK, 128), F32),
            pltpu.VMEM((1, max(NR, 1) * DH, 8 * PK, 128), F32),
            pltpu.VMEM((1, max(NR, 1) * DH, 8 * PK, 128), F32),
            pltpu.SMEM((1,), jnp.int32),
            pltpu.SemaphoreType.DMA((14,)),
            pltpu.SemaphoreType.DMA((NOC,)),
        ] + [pltpu.VMEM((1, DH, 8, 128), F32)] * 8 + [pltpu.VMEM((1, TK, 512), F32)] * (2 * NC) + [pltpu.VMEM((DH, D), BF16)] * 2 + [pltpu.VMEM((8, 128), F32)] * 0,
        compiler_params=pltpu.CompilerParams(vmem_limit_bytes=110 * 1024 * 1024),
        name="mha_mqa",
    )(A_x.reshape(S, D), A_wqkv, A_wo, B_x.reshape(S, D), B_wq, B_wk.T, B_wv.T, B_wo)
    return out.reshape(1, S, 2 * D)
```

```python
import math
import jax
import jax.numpy as jnp
from jax import lax
import jax.experimental.pallas as pl
import jax.experimental.pallas.tpu as pltpu

S = 2048
D = 640
H = 32
DH = 20
TK = 128
NC = S // TK
NQB = 16
NU = 2 * H * 4
NH = 12
NPRE = 3
XC = 512
NXC = S // XC
OC = 256
NOC = S // OC
QSCALE = (DH ** -0.5) * math.log2(math.e)

X = 12
NV = 16 * X
NM = S - NV
PK = 11
DS = 4
T0 = -50
T1 = 100
TS = 80
GD = 400
NPG = 5
PGD = 600
LJ = 9
NOMAX = 0
NOPROD = 0
FAST = 0
ROT = 1
_g16 = NM // 16
EV = 0
MSZ = ([16 * (((c + 1) * _g16) // NC - (c * _g16) // NC) for c in range(NC)] if EV else
       [16 * (_g16 // NC + (1 if c < _g16 % NC else 0)) for c in range(NC)])
MOFF = [NV + sum(MSZ[:c]) for c in range(NC)]
NR = -(-(NV // 8) // PK)
SLOT = 24 + NM // NC

def keep(r, d, j):
    return d == DH - 1 or (j + d // DS) % ROT == 0


_NT = (((1,), (1,)), ((), ()))
_TN = (((0,), (0,)), ((), ()))
F32 = jnp.float32
BF16 = jnp.bfloat16


def _kernel(ax_h, awqkv_h, awo_h, bx_h, bwq_h, bwkt_h, bwvt_h, bwo_h, out_h,
            ax, awqkv, awo, bx, bwq, bwo, outv,
            lhs_a, lhs_b, kp, qt, vt, ot, kb0, kb1, kb2, zero_ref, sem, osem, *rest):
    qss = (rest[0:4], rest[4:8])
    rest = rest[8:]
    sbufs, (bwkt, bwvt) = rest[:2 * NC], rest[2 * NC:2 * NC + 2]
    bufs = (sbufs[:NC], sbufs[NC:])
    kbs = (kb0, kb1, kb2)

    def cp(src, dst, k):
        return pltpu.make_async_copy(src, dst, sem.at[k])

    def xrows(i):
        return pl.ds(i * XC, XC)

    c_bwq = cp(bwq_h, bwq, 0)
    c_bwk = cp(bwkt_h, bwkt, 1)
    c_bwv = cp(bwvt_h, bwvt, 2)
    c_bx = [cp(bx_h.at[xrows(i)], bx.at[xrows(i)], 3 + i) for i in range(NXC)]
    c_awqkv = cp(awqkv_h, awqkv, 7)
    c_ax = [cp(ax_h.at[xrows(i)], ax.at[xrows(i)], 8 + i) for i in range(NXC)]
    c_awo = cp(awo_h, awo, 12)
    c_bwo = cp(bwo_h, bwo, 13)

    c_bwq.start()
    c_bwk.start()
    c_bwv.start()
    c_bx[0].start()
    zero_ref[0] = 0
    for padr in rest[2 * NC + 2:]:
        padr[...] = jnp.zeros((8, 128), F32)

    z = lambda r, c, dt: jnp.zeros((r, c), dt)

    c_bwq.wait()
    c_bwk.wait()
    c_bwv.wait()
    for i in range(1, NXC):
        c_bx[i].start()
    c_awqkv.start()
    lhs_b[0:D, :] = bwq[...].T
    wv = bwvt[...].astype(F32)
    wk = bwkt[...].astype(F32)
    lhs_b[D:D + 48, :] = jnp.concatenate([wv, z(4, D, F32), wk, z(4, D, F32)], axis=0).astype(BF16)

    def prep_a():
        lhs_a[0:D, :] = awqkv[:, 0:D].T
        lhs_a[D:2 * D, :] = awqkv[:, 2 * D:3 * D].T

    def store_q(r, br, qb0):
        q = r * QSCALE
        for h in range(H):
            blk = jnp.concatenate([q[DH * h:DH * (h + 1)], z(12, XC, F32)], axis=0).astype(BF16)
            blk = pltpu.bitcast(blk, F32)
            for j in range(XC // 128):
                qt[(br * H + h) * NQB + qb0 + j] = blk[:, j * 128:(j + 1) * 128]

    def store_v(rows20, hidx, c0):
        vv = jnp.concatenate([rows20, jnp.ones((4, XC), F32)], axis=0)
        for j in range(XC // 128):
            vt[hidx, c0 + j, 0:24, :] = vv[:, j * 128:(j + 1) * 128]

    def proj_b(i):
        xc = bx[xrows(i), :]
        r = lax.dot_general(lhs_b[0:D + 48, :], xc, _NT, preferred_element_type=F32)
        store_q(r[0:D], 1, i * (XC // 128))
        store_v(r[D:D + DH], H, i * (XC // 128))
        k = jnp.concatenate([r[D + 24:D + 48], z(104, XC, F32)], axis=0).T.astype(BF16)
        kp[H, pl.ds(i * (XC // 2), XC // 2), :] = pltpu.bitcast(k, F32)

    for i in range(NXC):
        c_bx[i].wait()
        if i == 0:
            for k in range(NXC):
                c_ax[k].start()
        if i == NXC - 1:
            c_awqkv.wait()
            c_awo.start()
            c_bwo.start()
            prep_a()
        if not FAST:
            proj_b(i)

    for k in range(NXC):
        c_ax[k].wait()

    lane = lax.broadcasted_iota(jnp.int32, (64, 128), 1)

    def proj_a(i, c):
        rows = pl.ds(pl.multiple_of(i * XC, XC), XC)
        xc = ax[rows, :]
        for j in range(XC // 128):
            k = jnp.dot(xc[j * 128:(j + 1) * 128], awqkv[:, D:2 * D], preferred_element_type=F32).astype(BF16)
            k = pltpu.bitcast(k, F32)
            for h in range(H):
                t, off = divmod(DH * h, 128)
                win = k[:, 128 * t:128 * (t + 1)]
                if off:
                    win = pltpu.roll(win, 128 - off, 1)
                if off + DH > 128:
                    nxt = pltpu.roll(k[:, 128 * (t + 1):128 * (t + 2)], 128 - off, 1)
                    win = jnp.where(lane < 128 - off, win, nxt)
                kp[h, pl.ds(pl.multiple_of(i * (XC // 2) + j * 64, 64), 64), :] = win
        r = lax.dot_general(lhs_a[...], xc, _NT, preferred_element_type=F32)
        store_q(r[0:D], 0, i * (XC // 128))
        for h in range(H):
            store_v(r[D + DH * h:D + DH * (h + 1)], h, i * (XC // 128))
        return c
    if not FAST:
        lax.fori_loop(0, NXC, proj_a, 0)

    def st(buf, r0, n, v, val):
        o = 0
        while o < n:
            c, rr = divmod(r0 + o, TK)
            k = min(n - o, TK - rr)
            buf[c][0, rr:rr + k, v * 128:(v + 1) * 128] = val[o:o + k]
            o += k

    def produce(kidx, kb, g, d0, d1, flag, gate):
        k32 = kp[kidx, 8 * g:8 * (g + 1), :]
        if gate is not None:
            k32 = jnp.where(flag, gate, k32)
        kf = pltpu.bitcast(k32, BF16).astype(F32)
        for d in range(d0, d1):
            bc = jnp.broadcast_to(kf[:, d:d + 1], (16, 128))
            for r in range(2):
                pr, a = divmod(2 * g + r, PK)
                kb[0, pr * DH + d, 8 * a:8 * (a + 1), :] = bc[8 * r:8 * (r + 1)]

    class P1:
        def __init__(self, u, s, off):
            bh = u // 4
            self.bh = bh
            self.kidx = jnp.minimum(bh, H)
            self.qc = qc = s % 4
            self.hs = s // 4
            self.off = off and X > 0
            self.msz = MSZ if self.off else [TK] * NC
            self.moff = MOFF if self.off else [TK * c for c in range(NC)]
            self.qblk = [pltpu.bitcast(qt[bh * NQB + qc * 4 + v], BF16) for v in range(4)]
            self.w = [jnp.concatenate([b, z(96, 128, BF16)], axis=0) for b in self.qblk]
            self.mx = [None] * 4
            self.mv = [None] * 4
            self.buf = bufs[s % 2]
            self.qs = qss[s % 2]

        def upd(self, v, val):
            self.mx[v] = val if self.mx[v] is None else jnp.maximum(self.mx[v], val)

        def build(self, v, zoff, flag, gate):
            kb = kbs[self.hs % 3]
            qs = self.qs[v]
            qf = self.qblk[v].astype(F32)
            for d in range(DH):
                row = jnp.broadcast_to(qf[d:d + 1], (8, 128))
                if d == 0 and gate is not None:
                    row = jnp.where(flag, gate, row)
                qs[0, d] = row
            vals = []
            for r in range(NR):
                n = min(PK, NV // 8 - r * PK)
                acc = None
                for d in range(DH):
                    t = kb[zoff, r * DH + d, 0:8 * n, :].reshape(n, 8, 128) * qs[zoff, d][None]
                    acc = t if acc is None else acc + t
                    if (d + 1) % DS == 0:
                        vals += [acc[j] for j in range(n) if keep(r, d, j)]
                st(self.buf, r * PK * 8, 8 * n, v, acc.reshape(8 * n, 128))
                am = jnp.max(acc, axis=0)
                self.mv[v] = am if self.mv[v] is None else jnp.maximum(self.mv[v], am)
            return vals

        def chunk(self, c, v, flag, anch):
            kc = kp[self.kidx, pl.ds(self.moff[c] // 2, self.msz[c] // 2), :]
            if anch:
                parts = []
                for j in range(self.msz[c] // 16):
                    p32 = kc[8 * j:8 * (j + 1)]
                    for val in anch.get(j, []):
                        p32 = jnp.where(flag, val, p32)
                    parts.append(p32)
                kc = jnp.concatenate(parts, axis=0)
            s = jnp.dot(pltpu.bitcast(kc, BF16), self.w[v], preferred_element_type=F32)
            st(self.buf, self.moff[c], self.msz[c], v, s)
            self.upd(v, jnp.max(s.reshape(self.msz[c] // 8, 8, 128), axis=0))
            return s[0:8]

        def finish(self, v):
            if NOMAX:
                return jnp.zeros((1, 128), F32)
            m = jnp.maximum(self.mx[v], self.mv[v]) if self.off else self.mx[v]
            return jnp.max(m, axis=0, keepdims=True)

    class P2:
        def __init__(self, u, qc, par, zoff):
            self.bh = u // 4
            self.qc = qc
            self.vidx = jnp.minimum(self.bh, H)
            self.acc = [None] * 4
            self.buf, self.zoff = bufs[par], zoff

        def chunk(self, c, v, m):
            if NOMAX:
                p = jnp.exp2(self.buf[c][self.zoff, :, v * 128:(v + 1) * 128])
            else:
                p = jnp.exp2(self.buf[c][self.zoff, :, v * 128:(v + 1) * 128] - m)
            d = jnp.dot(vt[self.vidx, c, 0:24, :], p, preferred_element_type=F32,
                        precision=lax.Precision.DEFAULT)
            self.acc[v] = d if self.acc[v] is None else self.acc[v] + d
            if c == NC - 1:
                a = self.acc[v]
                br, h = self.bh // H, self.bh % H
                ot[br * NQB + self.qc * 4 + v, pl.ds(pl.multiple_of(h * 24, 8), 24), :] = a * (1.0 / a[23:24, :])

    def run(u0, s0, n1, n2, m, zoff, extra=()):
        ms = {}
        if m is not None:
            for v in range(4):
                ms[(0, v)] = m[:, v * 128:(v + 1) * 128]
        p1s, p2s = {}, {}
        lag = LJ if n1 else 0
        extra = list(extra)
        flag = (jnp.full((8, 128), zoff, jnp.int32) != 0) if n1 else None

        def getp1(t):
            if t not in p1s:
                p1s[t] = P1(u0 + t + 1, s0 + t + 1, s0 + t + 1 > 0)
            return p1s[t]

        njobs = n1 * NC * 4
        jt = lambda n: n * SLOT // 4
        nj = lambda n: (MSZ if s0 + n // (4 * NC) + 1 > 0 else [TK] * NC)[(n // 4) % NC] // 16
        pts = sorted((jt(n) + 16 * j, n, j) for n in range(njobs) for j in range(nj(n)))
        builds = {}
        anchors = {}
        gates = {}
        L = SLOT * NC
        per_col = sum(1 for r in range(NR) for d in range(DS - 1, DH, DS) for j in range(min(PK, NV // 8 - r * PK)) if keep(r, d, j))
        for t in range(n1):
            if not X:
                break
            if s0 + t + 1 > 0:
                w = [p for p in pts if max(t * L + T0, TS) <= p[0] <= (t + 1) * L - T1]
                for v in range(4):
                    mine = [w[(v * per_col + i) * len(w) // (4 * per_col)] for i in range(per_col)]
                    first = min(p[1] for p in mine)
                    gj = max([n for n in range(first) if jt(n) <= mine[0][0] - GD], default=None)

                    def bld(t=t, v=v, mine=mine, gj=gj):
                        vals = getp1(t).build(v, zoff, flag, None if gj is None else gates[gj])
                        for val, p in zip(vals, mine):
                            anchors.setdefault(p[1], {}).setdefault(p[2], []).append(val)
                    builds.setdefault(first, []).append(bld)
            s = s0 + t + 1
            grp = [(s // 4 + 1, g, k) for g in range(X * (s % 4) // 4, X * (s % 4 + 1) // 4) for k in range(NPG)]
            if s == 0:
                grp = [(0, g, k) for g in range(X) for k in range(NPG)] + grp
            w = [p for p in pts if max(t * L, TS + 100) <= p[0] <= (t + 1) * L - 300]
            for i, (hs, g, k) in enumerate(grp if not NOPROD else []):
                p = w[(2 * i + 1) * len(w) // (2 * len(grp))]

                gj = max([n for n in range(p[1]) if jt(n) <= p[0] - PGD], default=None)

                def prod(t=t, hs=hs, g=g, k=k, p=p, s=s, gj=gj):
                    kidx = jnp.minimum(getp1(t).bh + (hs - s // 4), H)
                    produce(kidx, kbs[hs % 3], g, DH * k // NPG, DH * (k + 1) // NPG,
                            flag, None if gj is None else gates[gj])
                    pr, a = divmod(2 * g, PK)
                    val = kbs[hs % 3][zoff, pr * DH + DH * k // NPG, 8 * a:8 * (a + 1), :]
                    anchors.setdefault(p[1], {}).setdefault(p[2], []).append(val)
                builds.setdefault(p[1], []).append(prod)

        for n in range(max(njobs, n2 * NC * 4 + lag)):
            if n < njobs:
                t, c, vi = n // (4 * NC), (n // 4) % NC, n % 4
                for f in builds.get(n, []):
                    f()
                gates[n] = getp1(t).chunk(c, vi, flag, anchors.get(n))
                if c == NC - 1:
                    ms[(t + 1, vi)] = p1s[t].finish(vi)
            n_ = n - lag
            if 0 <= n_ < n2 * NC * 4:
                t, c, v = n_ // (4 * NC), (n_ // 4) % NC, n_ % 4
                if t not in p2s:
                    p2s[t] = P2(u0 + t, (s0 + t) % 4, (s0 + t) % 2, zoff)
                p2s[t].chunk(c, v, ms[(t, v)])
            if extra and n % 4 == 3:
                extra.pop(0)()
        for f in extra:
            f()
        if n1:
            return jnp.concatenate([ms[(n1, v)] for v in range(4)], axis=1)

    zoff0 = zero_ref[0]
    if FAST:
        m0 = jnp.zeros((1, 512), F32)
    else:
        m0 = run(-1, -1, 1, 0, None, zoff0)
        m0 = run(0, 0, NPRE, NPRE, m0, zoff0)

    def body(i, m):
        return run(NPRE + i * NH, NPRE, NH, NH, m, zero_ref[0])
    m_last = lax.fori_loop(0, (NU - 1 - NPRE) // NH, body, m0)

    c_awo.wait()
    c_bwo.wait()

    def ocopy(i):
        rows = pl.ds(i * OC, OC)
        return pltpu.make_async_copy(outv.at[rows], out_h.at[rows], osem.at[i])

    def o_t(br, qb):
        o24 = ot[br * NQB + qb]
        return jnp.concatenate([o24[24 * h:24 * h + DH] for h in range(H)], axis=0).astype(BF16)

    def oproj(i):
        rows = pl.ds(i * OC, OC)
        for br, wo in ((0, awo), (1, bwo)) if not FAST else ():
            o = jnp.concatenate([o_t(br, i * (OC // 128) + j) for j in range(OC // 128)], axis=1)
            res = lax.dot_general(o, wo[...], _TN, preferred_element_type=F32)
            outv[rows, br * D:(br + 1) * D] = res.astype(BF16)
        ocopy(i).start()

    pieces = []
    for br, wo in ((0, awo), (1, bwo)):
        for j in range(OC // 128):
            o_n = o_t(br, j).T
            for n in range(D // 128):
                def piece(br=br, wo=wo, j=j, n=n, o_n=o_n):
                    res = jnp.dot(o_n, wo[:, n * 128:(n + 1) * 128], preferred_element_type=F32)
                    outv[j * 128:(j + 1) * 128, br * D + n * 128:br * D + (n + 1) * 128] = res.astype(BF16)
                pieces.append(piece)
    run(NU - 1, 3, 0, 1, m_last, 0, extra=pieces)
    ocopy(0).start()
    for i in range(1, NOC):
        oproj(i)
    for i in range(NOC):
        ocopy(i).wait()


@jax.jit
def pallas_concat_heads__softmax_full_mha__grouped_kv_mqa__prompt_kernel(
    A_x, A_wqkv, A_wo, B_x, B_wq, B_wk, B_wv, B_wo,
):
    anyspec = pl.BlockSpec(memory_space=pl.ANY)
    out = pl.pallas_call(
        _kernel,
        out_shape=jax.ShapeDtypeStruct((S, 2 * D), BF16),
        in_specs=[anyspec] * 8,
        out_specs=anyspec,
        scratch_shapes=[
            pltpu.VMEM((S, D), BF16),
            pltpu.VMEM((D, 3 * D), BF16),
            pltpu.VMEM((D, D), BF16),
            pltpu.VMEM((S, D), BF16),
            pltpu.VMEM((D, D), BF16),
            pltpu.VMEM((D, D), BF16),
            pltpu.VMEM((S, 2 * D), BF16),
            pltpu.VMEM((2 * D, D), BF16),
            pltpu.VMEM((D + 64, D), BF16),
            pltpu.VMEM((H + 1, S // 2, 128), F32),
            pltpu.VMEM((2 * H * NQB, 16, 128), F32),
            pltpu.VMEM((H + 1, NC, 32, 128), F32),
            pltpu.VMEM((2 * NQB, H * 24, 128), F32),
            pltpu.VMEM((1, max(NR, 1) * DH, 8 * PK, 128), F32),
            pltpu.VMEM((1, max(NR, 1) * DH, 8 * PK, 128), F32),
            pltpu.VMEM((1, max(NR, 1) * DH, 8 * PK, 128), F32),
            pltpu.SMEM((1,), jnp.int32),
            pltpu.SemaphoreType.DMA((14,)),
            pltpu.SemaphoreType.DMA((NOC,)),
        ] + [pltpu.VMEM((1, DH, 8, 128), F32)] * 8 + [pltpu.VMEM((1, TK, 512), F32)] * (2 * NC) + [pltpu.VMEM((DH, D), BF16)] * 2 + [pltpu.VMEM((8, 128), F32)] * 0,
        compiler_params=pltpu.CompilerParams(vmem_limit_bytes=110 * 1024 * 1024),
        name="mha_mqa",
    )(A_x.reshape(S, D), A_wqkv, A_wo, B_x.reshape(S, D), B_wq, B_wk.T, B_wv.T, B_wo)
    return out.reshape(1, S, 2 * D)
```

```python
import math

import jax
import jax.numpy as jnp
from jax import lax
import jax.experimental.pallas as pl
import jax.experimental.pallas.tpu as pltpu

S = 2048
D = 640
H = 32
DH = 20
TK = 128
NC = S // TK
NQB = 16
NU = 2 * H * 4
NH = 12
NPRE = 3
XC = 512
NXC = S // XC
OCH = [(0, 2), (2, 2), (4, 2), (6, 2), (8, 2), (10, 2), (12, 2), (14, 1), (15, 1)]
NOC = len(OCH)
QSCALE = (DH ** -0.5) * math.log2(math.e)

X = 13
NV = 16 * X
NM = S - NV
PK = 14
DS = 4
T0, T1, TS = -100, 100, 80
GD, PGD = 400, 600
NPG = 5
LJ = 9
_g16 = NM // 16
MSZ = [16 * (_g16 // NC + (1 if c < _g16 % NC else 0)) for c in range(NC)]
MOFF = [NV + sum(MSZ[:c]) for c in range(NC)]
NR = -(-(NV // 8) // PK)
SLOT = 24 + NM // NC
ND = DH // DS
KBN = -(-(DS * PK + 2) // 4) * 4

_NT = (((1,), (1,)), ((), ()))
_TN = (((0,), (0,)), ((), ()))
F32 = jnp.float32
BF16 = jnp.bfloat16


def _kernel(ax_h, awqkv_h, awo_h, bx_h, bwq_h, bwkt_h, bwvt_h, bwo_h, out_h,
            ax, awqkv, awo, bx, bwq, bwo, outv,
            lhs_a, lhs_b, kp, qt, vt, ot, zero_ref, sem, osem, *rest):
    kbs = [[rest[(b * NR + r) * ND:(b * NR + r + 1) * ND] for r in range(NR)] for b in range(3)]
    rest = rest[3 * NR * ND:]
    qss = (rest[0:4], rest[4:8])
    rest = rest[8:]
    sbufs, (bwkt, bwvt) = rest[:2 * NC], rest[2 * NC:2 * NC + 2]
    bufs = (sbufs[:NC], sbufs[NC:])

    def cp(src, dst, k):
        return pltpu.make_async_copy(src, dst, sem.at[k])

    def xrows(i):
        return pl.ds(i * XC, XC)

    c_bwq = cp(bwq_h, bwq, 0)
    c_bwk = cp(bwkt_h, bwkt, 1)
    c_bwv = cp(bwvt_h, bwvt, 2)
    c_bx = [cp(bx_h.at[xrows(i)], bx.at[xrows(i)], 3 + i) for i in range(NXC)]
    c_awqkv = cp(awqkv_h, awqkv, 7)
    c_ax = [cp(ax_h.at[xrows(i)], ax.at[xrows(i)], 8 + i) for i in range(NXC)]
    c_awo = cp(awo_h, awo, 12)
    c_bwo = cp(bwo_h, bwo, 13)

    c_bwk.start()
    c_bwv.start()
    c_bwq.start()
    c_bx[0].start()
    zero_ref[0] = 0
    z = lambda r, c, dt: jnp.zeros((r, c), dt)

    c_bwk.wait()
    c_bwv.wait()
    c_bwq.wait()
    c_bx[1].start()
    lhs_b[48:48 + D, :] = bwq[...].T
    wv = bwvt[...].astype(F32)
    wk = bwkt[...].astype(F32)
    lhs_b[0:48, :] = jnp.concatenate([wk, z(4, D, F32), wv, z(4, D, F32)], axis=0).astype(BF16)

    def prep_a():
        lhs_a[0:D, :] = awqkv[:, 0:D].T
        lhs_a[D:2 * D, :] = awqkv[:, 2 * D:3 * D].T

    def store_q(r, br, qb0):
        q = r * QSCALE
        for h in range(H):
            blk = jnp.concatenate([q[DH * h:DH * (h + 1)], z(12, XC, F32)], axis=0).astype(BF16)
            blk = pltpu.bitcast(blk, F32)
            for j in range(XC // 128):
                qt[(br * H + h) * NQB + qb0 + j] = blk[:, j * 128:(j + 1) * 128]

    def store_v(rows20, hidx, c0):
        vv = jnp.concatenate([rows20, jnp.ones((4, XC), F32)], axis=0)
        for j in range(XC // 128):
            vt[hidx, c0 + j, 0:24, :] = vv[:, j * 128:(j + 1) * 128]

    def proj_b(i):
        xc = bx[xrows(i), :]
        r = lax.dot_general(lhs_b[0:D + 48, :], xc, _NT, preferred_element_type=F32)
        store_q(r[48:48 + D], 1, i * (XC // 128))
        store_v(r[24:24 + DH], H, i * (XC // 128))
        k = jnp.concatenate([r[0:24], z(104, XC, F32)], axis=0).T.astype(BF16)
        kp[H, pl.ds(i * (XC // 2), XC // 2), :] = pltpu.bitcast(k, F32)

    c_bx[0].wait()
    c_bx[2].start()
    c_bx[3].start()
    proj_b(0)
    c_bx[1].wait()
    c_awqkv.start()
    proj_b(1)
    c_bx[2].wait()
    c_bx[3].wait()
    for k in range(NXC):
        c_ax[k].start()
    proj_b(2)
    c_awqkv.wait()
    prep_a()
    proj_b(3)
    for k in range(NXC):
        c_ax[k].wait()
    c_awo.start()
    c_bwo.start()

    lane = lax.broadcasted_iota(jnp.int32, (64, 128), 1)

    def proj_a(i, c):
        rows = pl.ds(pl.multiple_of(i * XC, XC), XC)
        xc = ax[rows, :]
        for j in range(XC // 128):
            k = jnp.dot(xc[j * 128:(j + 1) * 128], awqkv[:, D:2 * D], preferred_element_type=F32).astype(BF16)
            k = pltpu.bitcast(k, F32)
            for h in range(H):
                t, off = divmod(DH * h, 128)
                win = k[:, 128 * t:128 * (t + 1)]
                if off:
                    win = pltpu.roll(win, 128 - off, 1)
                if off + DH > 128:
                    nxt = pltpu.roll(k[:, 128 * (t + 1):128 * (t + 2)], 128 - off, 1)
                    win = jnp.where(lane < 128 - off, win, nxt)
                kp[h, pl.ds(pl.multiple_of(i * (XC // 2) + j * 64, 64), 64), :] = win
        r = lax.dot_general(lhs_a[...], xc, _NT, preferred_element_type=F32)
        store_q(r[0:D], 0, i * (XC // 128))
        for h in range(H):
            store_v(r[D + DH * h:D + DH * (h + 1)], h, i * (XC // 128))
        return c
    lax.fori_loop(0, NXC, proj_a, 0)

    def st(buf, r0, n, v, val):
        o = 0
        while o < n:
            c, rr = divmod(r0 + o, TK)
            k = min(n - o, TK - rr)
            buf[c][0, rr:rr + k, v * 128:(v + 1) * 128] = val[o:o + k]
            o += k

    def produce(kidx, kb, g, d0, d1, flag, gate):
        k32 = kp[kidx, 8 * g:8 * (g + 1), :]
        if gate is not None:
            k32 = jnp.where(flag, gate, k32)
        kf = pltpu.bitcast(k32, BF16).astype(F32)
        for d in range(d0, d1):
            bc = jnp.broadcast_to(kf[:, d:d + 1], (16, 128))
            for r in range(2):
                pr, a = divmod(2 * g + r, PK)
                kb[pr][d // DS][0, (d % DS) * PK + a] = bc[8 * r:8 * (r + 1)]

    class P1:
        def __init__(self, u, s, off):
            bh = u // 4
            self.bh = bh
            self.kidx = jnp.minimum(bh, H)
            qc = s % 4
            self.hs = s // 4
            self.off = off
            self.msz = MSZ if off else [TK] * NC
            self.moff = MOFF if off else [TK * c for c in range(NC)]
            self.qblk = [pltpu.bitcast(qt[bh * NQB + qc * 4 + v], BF16) for v in range(4)]
            self.w = [jnp.concatenate([b, z(96, 128, BF16)], axis=0) for b in self.qblk]
            self.mx = [None] * 4
            self.mv = [None] * 4
            self.buf = bufs[s % 2]
            self.qs = qss[s % 2]

        def build(self, v, r, d0, zoff, flag, gate):
            qs = self.qs[v]
            if r == 0 and d0 == 0:
                qf = self.qblk[v].astype(F32)
                for d in range(DH):
                    row = jnp.broadcast_to(qf[d:d + 1], (8, 128))
                    if d == 0 and gate is not None:
                        row = jnp.where(flag, gate, row)
                    qs[0, d] = row
            n = min(PK, NV // 8 - r * PK)
            acc = self.acc if d0 else None
            ka = kbs[self.hs % 3][r][d0 // DS]
            for d in range(d0, d0 + DS):
                t = ka[zoff, (d - d0) * PK:(d - d0) * PK + n] * qs[zoff, d][None]
                acc = t if acc is None else acc + t
            self.acc = acc
            if d0 + DS == DH:
                st(self.buf, r * PK * 8, 8 * n, v, acc.reshape(8 * n, 128))
                am = jnp.max(acc, axis=0)
                self.mv[v] = am if self.mv[v] is None else jnp.maximum(self.mv[v], am)
            return [acc[j] for j in range(n)]

        def chunk(self, c, v, flag, anch):
            kc = kp[self.kidx, pl.ds(self.moff[c] // 2, self.msz[c] // 2), :]
            if anch:
                parts = []
                for j in range(self.msz[c] // 16):
                    p32 = kc[8 * j:8 * (j + 1)]
                    for val in anch.get(j, []):
                        p32 = jnp.where(flag, val, p32)
                    parts.append(p32)
                kc = jnp.concatenate(parts, axis=0)
            s = jnp.dot(pltpu.bitcast(kc, BF16), self.w[v], preferred_element_type=F32)
            st(self.buf, self.moff[c], self.msz[c], v, s)
            mc = jnp.max(s.reshape(self.msz[c] // 8, 8, 128), axis=0)
            self.mx[v] = mc if self.mx[v] is None else jnp.maximum(self.mx[v], mc)
            return s[0:8]

        def finish(self, v):
            m = jnp.maximum(self.mx[v], self.mv[v]) if self.off else self.mx[v]
            return jnp.max(m, axis=0, keepdims=True)

    class P2:
        def __init__(self, u, qc, par, zoff):
            self.bh = u // 4
            self.qc = qc
            self.vidx = jnp.minimum(self.bh, H)
            self.acc = [None] * 4
            self.buf, self.zoff = bufs[par], zoff

        def chunk(self, c, v, m):
            p = jnp.exp2(self.buf[c][self.zoff, :, v * 128:(v + 1) * 128] - m)
            d = jnp.dot(vt[self.vidx, c, 0:24, :], p, preferred_element_type=F32,
                        precision=lax.Precision.DEFAULT)
            self.acc[v] = d if self.acc[v] is None else self.acc[v] + d
            if c == NC - 1:
                a = self.acc[v]
                br, h = self.bh // H, self.bh % H
                ot[br * NQB + self.qc * 4 + v, pl.ds(pl.multiple_of(h * 24, 8), 24), :] = a * (1.0 / a[23:24, :])

    def run(u0, s0, n1, n2, m, zoff, extra=()):
        ms = {}
        if m is not None:
            for v in range(4):
                ms[(0, v)] = m[:, v * 128:(v + 1) * 128]
        p1s, p2s = {}, {}
        lag = LJ if n1 else 0
        extra = list(extra)
        flag = (jnp.full((8, 128), zoff, jnp.int32) != 0) if n1 else None

        def getp1(t):
            if t not in p1s:
                p1s[t] = P1(u0 + t + 1, s0 + t + 1, s0 + t + 1 > 0)
            return p1s[t]

        njobs = n1 * NC * 4
        jt = lambda n: n * SLOT // 4
        nj = lambda n: (MSZ if s0 + n // (4 * NC) + 1 > 0 else [TK] * NC)[(n // 4) % NC] // 16
        pts = sorted((jt(n) + 16 * j, n, j) for n in range(njobs) for j in range(nj(n)))
        builds = {}
        anchors = {}
        gates = {}
        L = SLOT * NC
        last_prod = {}
        for t in range(n1):
            s = s0 + t + 1
            if s > 0:
                w = [p for p in pts if max(t * L + T0, TS) <= p[0] <= (t + 1) * L - T1]
                subs = [(v, r, d0) for v in range(4) for r in range(NR) for d0 in range(0, DH, DS)]
                wt = [min(PK, NV // 8 - r * PK) for (v, r, d0) in subs]
                tot = sum(wt)
                mines = []
                pos = 0
                for n in wt:
                    mines.append([w[(pos + j) * len(w) // tot] for j in range(n)])
                    pos += n
                firsts = [min(p[1] for p in mine) for mine in mines]
                for k in range(len(firsts) - 2, -1, -1):
                    firsts[k] = min(firsts[k], firsts[k + 1])
                assert firsts[0] > last_prod.get(s // 4, -1)
                assert firsts[-1] <= (t + 1) * 4 * NC - 4
                for (v, r, d0), mine, first in zip(subs, mines, firsts):
                    gj = max([n for n in range(first) if jt(n) <= mine[0][0] - GD], default=None)

                    def bld(t=t, v=v, r=r, d0=d0, mine=mine, gj=gj):
                        vals = getp1(t).build(v, r, d0, zoff, flag, None if gj is None else gates[gj])
                        for val, p in zip(vals, mine):
                            anchors.setdefault(p[1], {}).setdefault(p[2], []).append(val)
                    builds.setdefault(first, []).append(bld)
            grp = [(s // 4 + 1, g, k) for g in range(X * (s % 4) // 4, X * (s % 4 + 1) // 4) for k in range(NPG)]
            if s == 0:
                grp = [(0, g, k) for g in range(X) for k in range(NPG)] + grp
            w = [p for p in pts if max(t * L, TS + 100) <= p[0] <= (t + 1) * L - 300]
            for i, (hs, g, k) in enumerate(grp):
                p = w[(2 * i + 1) * len(w) // (2 * len(grp))]
                gj = max([n for n in range(p[1]) if jt(n) <= p[0] - PGD], default=None)

                def prod(t=t, hs=hs, g=g, k=k, p=p, s=s, gj=gj):
                    kidx = jnp.minimum(getp1(t).bh + (hs - s // 4), H)
                    produce(kidx, kbs[hs % 3], g, DH * k // NPG, DH * (k + 1) // NPG,
                            flag, None if gj is None else gates[gj])
                    pr, a = divmod(2 * g, PK)
                    dd = DH * k // NPG
                    val = kbs[hs % 3][pr][dd // DS][zoff, (dd % DS) * PK + a]
                    anchors.setdefault(p[1], {}).setdefault(p[2], []).append(val)
                builds.setdefault(p[1], []).append(prod)
                last_prod[hs] = max(last_prod.get(hs, -1), p[1])

        for n in range(max(njobs, n2 * NC * 4 + lag)):
            if n < njobs:
                t, c, vi = n // (4 * NC), (n // 4) % NC, n % 4
                for f in builds.get(n, []):
                    f()
                gates[n] = getp1(t).chunk(c, vi, flag, anchors.get(n))
                if c == NC - 1:
                    ms[(t + 1, vi)] = p1s[t].finish(vi)
            n_ = n - lag
            if 0 <= n_ < n2 * NC * 4:
                t, c, v = n_ // (4 * NC), (n_ // 4) % NC, n_ % 4
                if t not in p2s:
                    p2s[t] = P2(u0 + t, (s0 + t) % 4, (s0 + t) % 2, zoff)
                p2s[t].chunk(c, v, ms[(t, v)])
            if extra and n % 4 == 3:
                extra.pop(0)()
        for f in extra:
            f()
        if n1:
            return jnp.concatenate([ms[(n1, v)] for v in range(4)], axis=1)

    zoff0 = zero_ref[0]
    m0 = run(-1, -1, 1, 0, None, zoff0)
    m0 = run(0, 0, NPRE, NPRE, m0, zoff0)

    def body(i, m):
        return run(NPRE + i * NH, NPRE, NH, NH, m, zero_ref[0])
    m_last = lax.fori_loop(0, (NU - 1 - NPRE) // NH, body, m0)

    c_awo.wait()
    c_bwo.wait()

    def ocopy(i):
        rows = pl.ds(OCH[i][0] * 128, OCH[i][1] * 128)
        return pltpu.make_async_copy(outv.at[rows], out_h.at[rows], osem.at[i])

    def o_t(br, qb):
        o24 = ot[br * NQB + qb]
        return jnp.concatenate([o24[24 * h:24 * h + DH] for h in range(H)], axis=0).astype(BF16)

    def oproj(i):
        rows = pl.ds(OCH[i][0] * 128, OCH[i][1] * 128)
        for br, wo in ((0, awo), (1, bwo)):
            o = jnp.concatenate([o_t(br, OCH[i][0] + j) for j in range(OCH[i][1])], axis=1)
            res = lax.dot_general(o, wo[...], _TN, preferred_element_type=F32)
            outv[rows, br * D:(br + 1) * D] = res.astype(BF16)
        ocopy(i).start()

    pieces = []
    for br, wo in ((0, awo), (1, bwo)):
        for j in range(OCH[0][1]):
            o_n = o_t(br, j).T
            for n in range(D // 128):
                def piece(br=br, wo=wo, j=j, n=n, o_n=o_n):
                    res = jnp.dot(o_n, wo[:, n * 128:(n + 1) * 128], preferred_element_type=F32)
                    outv[j * 128:(j + 1) * 128, br * D + n * 128:br * D + (n + 1) * 128] = res.astype(BF16)
                pieces.append(piece)
    run(NU - 1, 3, 0, 1, m_last, 0, extra=pieces)
    ocopy(0).start()
    for i in range(1, NOC):
        oproj(i)
    for i in range(NOC):
        ocopy(i).wait()


@jax.jit
def pallas_concat_heads__softmax_full_mha__grouped_kv_mqa__prompt_kernel(
    A_x: jax.Array,
    A_wqkv: jax.Array,
    A_wo: jax.Array,
    B_x: jax.Array,
    B_wq: jax.Array,
    B_wk: jax.Array,
    B_wv: jax.Array,
    B_wo: jax.Array,
):
    anyspec = pl.BlockSpec(memory_space=pl.ANY)
    scratch = [
        pltpu.VMEM((S, D), BF16),
        pltpu.VMEM((D, 3 * D), BF16),
        pltpu.VMEM((D, D), BF16),
        pltpu.VMEM((S, D), BF16),
        pltpu.VMEM((D, D), BF16),
        pltpu.VMEM((D, D), BF16),
        pltpu.VMEM((S, 2 * D), BF16),
        pltpu.VMEM((2 * D, D), BF16),
        pltpu.VMEM((D + 64, D), BF16),
        pltpu.VMEM((H + 1, S // 2, 128), F32),
        pltpu.VMEM((2 * H * NQB, 16, 128), F32),
        pltpu.VMEM((H + 1, NC, 32, 128), F32),
        pltpu.VMEM((2 * NQB, H * 24, 128), F32),
        pltpu.SMEM((1,), jnp.int32),
        pltpu.SemaphoreType.DMA((14,)),
        pltpu.SemaphoreType.DMA((NOC,)),
    ]
    scratch += [pltpu.VMEM((1, KBN, 8, 128), F32)] * (3 * NR * ND)
    scratch += [pltpu.VMEM((1, DH, 8, 128), F32)] * 8
    scratch += [pltpu.VMEM((1, TK, 512), F32)] * (2 * NC)
    scratch += [pltpu.VMEM((DH, D), BF16)] * 2
    out = pl.pallas_call(
        _kernel,
        out_shape=jax.ShapeDtypeStruct((S, 2 * D), BF16),
        in_specs=[anyspec] * 8,
        out_specs=anyspec,
        scratch_shapes=scratch,
        compiler_params=pltpu.CompilerParams(vmem_limit_bytes=110 * 1024 * 1024),
        name="mha_mqa",
    )(A_x.reshape(S, D), A_wqkv, A_wo, B_x.reshape(S, D), B_wq, B_wk.T, B_wv.T, B_wo)
    return out.reshape(1, S, 2 * D)
```

```python
import math

import jax
import jax.numpy as jnp
from jax import lax
import jax.experimental.pallas as pl
import jax.experimental.pallas.tpu as pltpu

S = 2048
D = 640
H = 32
DH = 20
TK = 128
NC = S // TK
NQB = 16
NU = 2 * H * 4
NH = 12
NPRE = 3
XC = 512
NXC = S // XC
OCH = [(0, 2), (2, 2), (4, 2), (6, 2), (8, 2), (10, 2), (12, 2), (14, 1), (15, 1)]
NOC = len(OCH)
QSCALE = (DH ** -0.5) * math.log2(math.e)

X = 13
NV = 16 * X
NM = S - NV
PK = 13
DS = 5
T0, T1, TS = -75, 70, 80
GD, PGD = 400, 600
NPG = 5
LJ = 9
_g16 = NM // 16
DJ = 14
MR = 2
PS, PE = 500, 300
CR = 1
MSZ = [16 * (_g16 // NC + (1 if (c - MR) % NC < _g16 % NC else 0)) for c in range(NC)]
MOFF = [NV + sum(MSZ[:c]) for c in range(NC)]
NR = -(-(NV // 8) // PK)
SLOT = 24 + NM // NC
ND = DH // DS
KBN = -(-(DS * PK + 2) // 4) * 4

_NT = (((1,), (1,)), ((), ()))
_TN = (((0,), (0,)), ((), ()))
F32 = jnp.float32
BF16 = jnp.bfloat16


def _kernel(ax_h, awqkv_h, awo_h, bx_h, bwq_h, bwkt_h, bwvt_h, bwo_h, out_h,
            ax, awqkv, awo, bx, bwq, bwo, outv,
            lhs_a, lhs_b, kp, qt, vt, ot, rls, zero_ref, sem, osem, *rest):
    kbs = [[rest[(b * NR + r) * ND:(b * NR + r + 1) * ND] for r in range(NR)] for b in range(3)]
    rest = rest[3 * NR * ND:]
    qss = (rest[0:4], rest[4:8])
    rest = rest[8:]
    sbufs, (bwkt, bwvt) = rest[:2 * NC], rest[2 * NC:2 * NC + 2]
    bufs = (sbufs[:NC], sbufs[NC:])

    def cp(src, dst, k):
        return pltpu.make_async_copy(src, dst, sem.at[k])

    def xrows(i):
        return pl.ds(i * XC, XC)

    c_bwq = cp(bwq_h, bwq, 0)
    c_bwk = cp(bwkt_h, bwkt, 1)
    c_bwv = cp(bwvt_h, bwvt, 2)
    c_bx = [cp(bx_h.at[xrows(i)], bx.at[xrows(i)], 3 + i) for i in range(NXC)]
    c_awqkv = cp(awqkv_h, awqkv, 7)
    c_ax = [cp(ax_h.at[xrows(i)], ax.at[xrows(i)], 8 + i) for i in range(NXC)]
    c_awo = cp(awo_h, awo, 12)
    c_bwo = cp(bwo_h, bwo, 13)

    c_bwk.start()
    c_bwv.start()
    c_bwq.start()
    c_bx[0].start()
    zero_ref[0] = 0
    z = lambda r, c, dt: jnp.zeros((r, c), dt)

    c_bwk.wait()
    c_bwv.wait()
    c_bwq.wait()
    c_bx[1].start()
    lhs_b[48:48 + D, :] = bwq[...].T
    wv = bwvt[...].astype(F32)
    wk = bwkt[...].astype(F32)
    lhs_b[0:48, :] = jnp.concatenate([wk, z(4, D, F32), wv, z(4, D, F32)], axis=0).astype(BF16)

    def prep_a():
        lhs_a[0:D, :] = awqkv[:, 0:D].T
        lhs_a[D:2 * D, :] = awqkv[:, 2 * D:3 * D].T

    def store_q(r, br, qb0):
        q = r * QSCALE
        for h in range(H):
            blk = jnp.concatenate([q[DH * h:DH * (h + 1)], z(12, XC, F32)], axis=0).astype(BF16)
            blk = pltpu.bitcast(blk, F32)
            for j in range(XC // 128):
                qt[(br * H + h) * NQB + qb0 + j] = blk[:, j * 128:(j + 1) * 128]

    def store_v(rows20, hidx, c0):
        vv = jnp.concatenate([rows20, jnp.ones((4, XC), F32)], axis=0)
        for j in range(XC // 128):
            vt[hidx, c0 + j, 0:24, :] = vv[:, j * 128:(j + 1) * 128]

    def proj_b(i):
        xc = bx[xrows(i), :]
        r = lax.dot_general(lhs_b[0:D + 48, :], xc, _NT, preferred_element_type=F32)
        store_q(r[48:48 + D], 1, i * (XC // 128))
        store_v(r[24:24 + DH], H, i * (XC // 128))
        k = jnp.concatenate([r[0:24], z(104, XC, F32)], axis=0).T.astype(BF16)
        kp[H, pl.ds(i * (XC // 2), XC // 2), :] = pltpu.bitcast(k, F32)

    c_bx[0].wait()
    c_bx[2].start()
    c_bx[3].start()
    proj_b(0)
    c_bx[1].wait()
    c_awqkv.start()
    proj_b(1)
    c_bx[2].wait()
    c_bx[3].wait()
    for k in range(NXC):
        c_ax[k].start()
    proj_b(2)
    c_awqkv.wait()
    prep_a()
    proj_b(3)
    for k in range(NXC):
        c_ax[k].wait()
    c_awo.start()
    c_bwo.start()

    lane = lax.broadcasted_iota(jnp.int32, (64, 128), 1)

    def proj_a(i, c):
        rows = pl.ds(pl.multiple_of(i * XC, XC), XC)
        xc = ax[rows, :]
        for j in range(XC // 128):
            k = jnp.dot(xc[j * 128:(j + 1) * 128], awqkv[:, D:2 * D], preferred_element_type=F32).astype(BF16)
            k = pltpu.bitcast(k, F32)
            for h in range(H):
                t, off = divmod(DH * h, 128)
                win = k[:, 128 * t:128 * (t + 1)]
                if off:
                    win = pltpu.roll(win, 128 - off, 1)
                if off + DH > 128:
                    nxt = pltpu.roll(k[:, 128 * (t + 1):128 * (t + 2)], 128 - off, 1)
                    win = jnp.where(lane < 128 - off, win, nxt)
                kp[h, pl.ds(pl.multiple_of(i * (XC // 2) + j * 64, 64), 64), :] = win
        r = lax.dot_general(lhs_a[...], xc, _NT, preferred_element_type=F32)
        store_q(r[0:D], 0, i * (XC // 128))
        for h in range(H):
            store_v(r[D + DH * h:D + DH * (h + 1)], h, i * (XC // 128))
        return c
    lax.fori_loop(0, NXC, proj_a, 0)

    def st(buf, r0, n, v, val):
        o = 0
        while o < n:
            c, rr = divmod(r0 + o, TK)
            k = min(n - o, TK - rr)
            buf[c][0, rr:rr + k, v * 128:(v + 1) * 128] = val[o:o + k]
            o += k

    def produce(kidx, kb, g, d0, d1, flag, gate):
        k32 = kp[kidx, 8 * g:8 * (g + 1), :]
        if gate is not None:
            k32 = jnp.where(flag, gate, k32)
        kf = pltpu.bitcast(k32, BF16).astype(F32)
        for d in range(d0, d1):
            bc = jnp.broadcast_to(kf[:, d:d + 1], (16, 128))
            for r in range(2):
                pr, a = divmod(2 * g + r, PK)
                kb[pr][d // DS][0, (d % DS) * PK + a] = bc[8 * r:8 * (r + 1)]

    class P1:
        def __init__(self, u, s, off):
            bh = u // 4
            self.bh = bh
            self.kidx = jnp.minimum(bh, H)
            qc = s % 4
            self.hs = s // 4
            self.off = off
            self.msz = MSZ if off else [TK] * NC
            self.moff = MOFF if off else [TK * c for c in range(NC)]
            self.qblk = [pltpu.bitcast(qt[bh * NQB + qc * 4 + v], BF16) for v in range(4)]
            self.w = [jnp.concatenate([b, z(96, 128, BF16)], axis=0) for b in self.qblk]
            self.mx = [None] * 4
            self.mv = [None] * 4
            self.buf = bufs[s % 2]
            self.qs = qss[s % 2]

        def build(self, v, r, d0, zoff, flag, gate):
            qs = self.qs[v]
            if r == 0 and d0 == 0:
                qf = self.qblk[v].astype(F32)
                for d in range(DH):
                    row = jnp.broadcast_to(qf[d:d + 1], (8, 128))
                    if d == 0 and gate is not None:
                        row = jnp.where(flag, gate, row)
                    qs[0, d] = row
            n = min(PK, NV // 8 - r * PK)
            acc = self.acc if d0 else None
            ka = kbs[self.hs % 3][r][d0 // DS]
            for d in range(d0, d0 + DS):
                t = ka[zoff, (d - d0) * PK:(d - d0) * PK + n] * qs[zoff, d][None]
                acc = t if acc is None else acc + t
            self.acc = acc
            if d0 + DS == DH:
                st(self.buf, r * PK * 8, 8 * n, v, acc.reshape(8 * n, 128))
                am = jnp.max(acc, axis=0)
                self.mv[v] = am if self.mv[v] is None else jnp.maximum(self.mv[v], am)
            return [acc[j] for j in range(n)]

        def chunk(self, c, v, flag, anch):
            kc = kp[self.kidx, pl.ds(self.moff[c] // 2, self.msz[c] // 2), :]
            if anch:
                parts = []
                for j in range(self.msz[c] // 16):
                    p32 = kc[8 * j:8 * (j + 1)]
                    for val in anch.get(j, []):
                        p32 = jnp.where(flag, val, p32)
                    parts.append(p32)
                kc = jnp.concatenate(parts, axis=0)
            s = jnp.dot(pltpu.bitcast(kc, BF16), self.w[v], preferred_element_type=F32)
            st(self.buf, self.moff[c], self.msz[c], v, s)
            mc = jnp.max(s.reshape(self.msz[c] // 8, 8, 128), axis=0)
            self.mx[v] = mc if self.mx[v] is None else jnp.maximum(self.mx[v], mc)
            return s[0:8]

        def finish(self, v):
            m = jnp.maximum(self.mx[v], self.mv[v]) if self.off else self.mx[v]
            return jnp.max(m, axis=0, keepdims=True)

    class P2:
        def __init__(self, u, qc, par, zoff):
            self.u = u
            self.bh = u // 4
            self.qc = qc
            self.vidx = jnp.minimum(self.bh, H)
            self.acc = [None] * 4
            self.buf, self.zoff = bufs[par], zoff

        def chunk(self, c, v, m):
            p = jnp.exp2(self.buf[c][self.zoff, :, v * 128:(v + 1) * 128] - m)
            d = jnp.dot(vt[self.vidx, c, 0:24, :], p, preferred_element_type=F32,
                        precision=lax.Precision.DEFAULT)
            self.acc[v] = d if self.acc[v] is None else self.acc[v] + d
            if c == NC - 1:
                a = self.acc[v]
                br, h = self.bh // H, self.bh % H
                ot[br * NQB + self.qc * 4 + v, pl.ds(pl.multiple_of(h * 24, 8), 24), :] = a

        def recip(self, flag, gate):
            row = lax.broadcasted_iota(jnp.int32, (8, 128), 0)
            l = self.acc[3][16:24]
            if gate is not None:
                l = jnp.where(flag, gate, l)
            for k in (2, 1, 0):
                l = jnp.where(row == 4 + k, self.acc[k][16:24], l)
            rls[self.u] = 1.0 / l

    def run(u0, s0, n1, n2, m, zoff, extra=()):
        ms = {}
        if m is not None:
            for v in range(4):
                ms[(0, v)] = m[:, v * 128:(v + 1) * 128]
        p1s, p2s = {}, {}
        lag = LJ if n1 else 0
        extra = list(extra)
        flag = (jnp.full((8, 128), zoff, jnp.int32) != 0) if n1 else None

        def getp1(t):
            if t not in p1s:
                p1s[t] = P1(u0 + t + 1, s0 + t + 1, s0 + t + 1 > 0)
            return p1s[t]

        njobs = n1 * NC * 4
        jt = lambda n: n * SLOT // 4
        nj = lambda n: (MSZ if s0 + n // (4 * NC) + 1 > 0 else [TK] * NC)[(n // 4) % NC] // 16
        pts = sorted((jt(n) + 16 * j, n, j) for n in range(njobs) for j in range(nj(n)))
        builds = {}
        anchors = {}
        gates = {}
        L = SLOT * NC
        later = {}
        last_prod = {}
        for t in range(n1):
            s = s0 + t + 1
            if s > 0:
                w = [p for p in pts if max(t * L + T0, TS) <= p[0] <= (t + 1) * L - T1]
                subs = [((v + CR) % 4, r, d0) for v in range(4) for r in range(NR) for d0 in range(0, DH, DS)]
                wt = [min(PK, NV // 8 - r * PK) for (v, r, d0) in subs]
                tot = sum(wt)
                mines = []
                pos = 0
                for n in wt:
                    mines.append([w[(pos + j) * len(w) // tot] for j in range(n)])
                    pos += n
                firsts = [min(p[1] for p in mine) for mine in mines]
                for k in range(len(firsts) - 2, -1, -1):
                    firsts[k] = min(firsts[k], firsts[k + 1])
                assert firsts[0] > last_prod.get(s // 4, -1)
                assert firsts[-1] <= (t + 1) * 4 * NC - 4
                for (v, r, d0), mine, first in zip(subs, mines, firsts):
                    gj = max([n for n in range(first) if jt(n) <= mine[0][0] - GD], default=None)

                    def bld(t=t, v=v, r=r, d0=d0, mine=mine, gj=gj):
                        vals = getp1(t).build(v, r, d0, zoff, flag, None if gj is None else gates[gj])
                        for val, p in zip(vals, mine):
                            anchors.setdefault(p[1], {}).setdefault(p[2], []).append(val)
                    builds.setdefault(first, []).append(bld)
            grp = [(s // 4 + 1, g, k) for g in range(X * (s % 4) // 4, X * (s % 4 + 1) // 4) for k in range(NPG)]
            if s == 0:
                grp = [(0, g, k) for g in range(X) for k in range(NPG)] + grp
            w = [p for p in pts if max(t * L + PS, TS + 100) <= p[0] <= (t + 1) * L - PE]
            for i, (hs, g, k) in enumerate(grp):
                p = w[(2 * i + 1) * len(w) // (2 * len(grp))]
                gj = max([n for n in range(p[1]) if jt(n) <= p[0] - PGD], default=None)

                def prod(t=t, hs=hs, g=g, k=k, p=p, s=s, gj=gj):
                    kidx = jnp.minimum(getp1(t).bh + (hs - s // 4), H)
                    produce(kidx, kbs[hs % 3], g, DH * k // NPG, DH * (k + 1) // NPG,
                            flag, None if gj is None else gates[gj])
                    pr, a = divmod(2 * g, PK)
                    dd = DH * k // NPG
                    val = kbs[hs % 3][pr][dd // DS][zoff, (dd % DS) * PK + a]
                    anchors.setdefault(p[1], {}).setdefault(p[2], []).append(val)
                builds.setdefault(p[1], []).append(prod)
                last_prod[hs] = max(last_prod.get(hs, -1), p[1])

        for n in range(max(njobs, n2 * NC * 4 + lag)):
            if n < njobs:
                t, c, vi = n // (4 * NC), (n // 4) % NC, n % 4
                for f in builds.get(n, []):
                    f()
                gates[n] = getp1(t).chunk(c, vi, flag, anchors.get(n))
                if c == NC - 1:
                    ms[(t + 1, vi)] = p1s[t].finish(vi)
            n_ = n - lag
            if 0 <= n_ < n2 * NC * 4:
                t, c, v = n_ // (4 * NC), (n_ // 4) % NC, n_ % 4
                if t not in p2s:
                    p2s[t] = P2(u0 + t, (s0 + t) % 4, (s0 + t) % 2, zoff)
                p2s[t].chunk(c, v, ms[(t, v)])
                if c == NC - 1 and v == 3:
                    if n + DJ < njobs:
                        later.setdefault(n + DJ, []).append(p2s[t])
                    else:
                        p2s[t].recip(None, None)
            for p2 in later.get(n, []):
                p2.recip(flag, gates[n])
            if extra and n % 4 == 3:
                extra.pop(0)()
        for f in extra:
            f()
        if n1:
            return jnp.concatenate([ms[(n1, v)] for v in range(4)], axis=1)

    zoff0 = zero_ref[0]
    m0 = run(-1, -1, 1, 0, None, zoff0)
    m0 = run(0, 0, NPRE, NPRE, m0, zoff0)

    def body(i, m):
        return run(NPRE + i * NH, NPRE, NH, NH, m, zero_ref[0])
    m_last = lax.fori_loop(0, (NU - 1 - NPRE) // NH, body, m0)

    c_awo.wait()
    c_bwo.wait()

    def ocopy(i):
        rows = pl.ds(OCH[i][0] * 128, OCH[i][1] * 128)
        return pltpu.make_async_copy(outv.at[rows], out_h.at[rows], osem.at[i])

    def o_t(br, qb):
        o24 = ot[br * NQB + qb]
        rl = lambda h: rls[(br * H + h) * 4 + qb // 4, 4 + qb % 4:5 + qb % 4, :]
        return jnp.concatenate([o24[24 * h:24 * h + DH] * rl(h) for h in range(H)], axis=0).astype(BF16)

    def oproj(i):
        rows = pl.ds(OCH[i][0] * 128, OCH[i][1] * 128)
        for br, wo in ((0, awo), (1, bwo)):
            o = jnp.concatenate([o_t(br, OCH[i][0] + j) for j in range(OCH[i][1])], axis=1)
            res = lax.dot_general(o, wo[...], _TN, preferred_element_type=F32)
            outv[rows, br * D:(br + 1) * D] = res.astype(BF16)
        ocopy(i).start()

    pieces = []
    for br, wo in ((0, awo), (1, bwo)):
        for j in range(OCH[0][1]):
            o_n = o_t(br, j).T
            for n in range(D // 128):
                def piece(br=br, wo=wo, j=j, n=n, o_n=o_n):
                    res = jnp.dot(o_n, wo[:, n * 128:(n + 1) * 128], preferred_element_type=F32)
                    outv[j * 128:(j + 1) * 128, br * D + n * 128:br * D + (n + 1) * 128] = res.astype(BF16)
                pieces.append(piece)
    run(NU - 1, 3, 0, 1, m_last, 0, extra=pieces)
    ocopy(0).start()
    for i in range(1, NOC):
        oproj(i)
    for i in range(NOC):
        ocopy(i).wait()


@jax.jit
def pallas_concat_heads__softmax_full_mha__grouped_kv_mqa__prompt_kernel(
    A_x: jax.Array,
    A_wqkv: jax.Array,
    A_wo: jax.Array,
    B_x: jax.Array,
    B_wq: jax.Array,
    B_wk: jax.Array,
    B_wv: jax.Array,
    B_wo: jax.Array,
):
    anyspec = pl.BlockSpec(memory_space=pl.ANY)
    scratch = [
        pltpu.VMEM((S, D), BF16),
        pltpu.VMEM((D, 3 * D), BF16),
        pltpu.VMEM((D, D), BF16),
        pltpu.VMEM((S, D), BF16),
        pltpu.VMEM((D, D), BF16),
        pltpu.VMEM((D, D), BF16),
        pltpu.VMEM((S, 2 * D), BF16),
        pltpu.VMEM((2 * D, D), BF16),
        pltpu.VMEM((D + 64, D), BF16),
        pltpu.VMEM((H + 1, S // 2, 128), F32),
        pltpu.VMEM((2 * H * NQB, 16, 128), F32),
        pltpu.VMEM((H + 1, NC, 32, 128), F32),
        pltpu.VMEM((2 * NQB, H * 24, 128), F32),
        pltpu.VMEM((NU, 8, 128), F32),
        pltpu.SMEM((1,), jnp.int32),
        pltpu.SemaphoreType.DMA((14,)),
        pltpu.SemaphoreType.DMA((NOC,)),
    ]
    scratch += [pltpu.VMEM((1, KBN, 8, 128), F32)] * (3 * NR * ND)
    scratch += [pltpu.VMEM((1, DH, 8, 128), F32)] * 8
    scratch += [pltpu.VMEM((1, TK, 512), F32)] * (2 * NC)
    scratch += [pltpu.VMEM((DH, D), BF16)] * 2
    out = pl.pallas_call(
        _kernel,
        out_shape=jax.ShapeDtypeStruct((S, 2 * D), BF16),
        in_specs=[anyspec] * 8,
        out_specs=anyspec,
        scratch_shapes=scratch,
        compiler_params=pltpu.CompilerParams(vmem_limit_bytes=110 * 1024 * 1024),
        name="mha_mqa",
    )(A_x.reshape(S, D), A_wqkv, A_wo, B_x.reshape(S, D), B_wq, B_wk.T, B_wv.T, B_wo)
    return out.reshape(1, S, 2 * D)
```

```python
import math

import jax
import jax.numpy as jnp
from jax import lax
import jax.experimental.pallas as pl
import jax.experimental.pallas.tpu as pltpu

S = 2048
D = 640
H = 32
DH = 20
TK = 128
NC = S // TK
NQB = 16
NU = 2 * H * 4
NH = 12
NPRE = 3
XC = 512
NXC = S // XC
OCH = [(0, 2), (2, 2), (4, 2), (6, 2), (8, 2), (10, 2), (12, 2), (14, 1), (15, 1)]
NOC = len(OCH)
QSCALE = (DH ** -0.5) * math.log2(math.e)

X = 13
NV = 16 * X
NM = S - NV
PK = 13
DS = 5
T0, T1, TS = -75, 70, 80
GD, PGD = 400, 600
LJ = 9
_g16 = NM // 16
DJ = 14
MR = 2
PS, PE = 500, 300
CR = 1
MSZ = [16 * (_g16 // NC + (1 if (c - MR) % NC < _g16 % NC else 0)) for c in range(NC)]
MOFF = [NV + sum(MSZ[:c]) for c in range(NC)]
NR = -(-(NV // 8) // PK)
SLOT = 24 + NM // NC
ND = DH // DS
KBN = -(-(DS * PK) // 4) * 4

_NT = (((1,), (1,)), ((), ()))
_TN = (((0,), (0,)), ((), ()))
F32 = jnp.float32
BF16 = jnp.bfloat16


def _kernel(ax_h, awqkv_h, awo_h, bx_h, bwq_h, bwkt_h, bwvt_h, bwo_h, out_h,
            ax, awqkv, awo, bx, bwq, bwo, outv,
            lhs_a, lhs_b, kp, qt, vt, ot, rls, zero_ref, sem, osem, *rest):
    kbs = [[rest[(b * NR + r) * ND:(b * NR + r + 1) * ND] for r in range(NR)] for b in range(3)]
    rest = rest[3 * NR * ND:]
    qss = (rest[0:4], rest[4:8])
    rest = rest[8:]
    sbufs, (bwkt, bwvt) = rest[:2 * NC], rest[2 * NC:2 * NC + 2]
    bufs = (sbufs[:NC], sbufs[NC:])

    def cp(src, dst, k):
        return pltpu.make_async_copy(src, dst, sem.at[k])

    def xrows(i):
        return pl.ds(i * XC, XC)

    c_bwq = cp(bwq_h, bwq, 0)
    c_bwk = cp(bwkt_h, bwkt, 1)
    c_bwv = cp(bwvt_h, bwvt, 2)
    c_bx = [cp(bx_h.at[xrows(i)], bx.at[xrows(i)], 3 + i) for i in range(NXC)]
    c_awqkv = cp(awqkv_h, awqkv, 7)
    c_ax = [cp(ax_h.at[xrows(i)], ax.at[xrows(i)], 8 + i) for i in range(NXC)]
    c_awo = cp(awo_h, awo, 12)
    c_bwo = cp(bwo_h, bwo, 13)

    c_bwk.start()
    c_bwv.start()
    c_bwq.start()
    c_bx[0].start()
    zero_ref[0] = 0
    z = lambda r, c, dt: jnp.zeros((r, c), dt)

    c_bwk.wait()
    c_bwv.wait()
    c_bwq.wait()
    c_bx[1].start()
    lhs_b[48:48 + D, :] = bwq[...].T
    wv = bwvt[...].astype(F32)
    wk = bwkt[...].astype(F32)
    lhs_b[0:48, :] = jnp.concatenate([wk, z(4, D, F32), wv, z(4, D, F32)], axis=0).astype(BF16)

    def prep_a():
        lhs_a[0:D, :] = awqkv[:, 0:D].T
        lhs_a[D:2 * D, :] = awqkv[:, 2 * D:3 * D].T

    def store_q(r, br, qb0):
        q = r * QSCALE
        for h in range(H):
            blk = jnp.concatenate([q[DH * h:DH * (h + 1)], z(12, XC, F32)], axis=0).astype(BF16)
            blk = pltpu.bitcast(blk, F32)
            qt[pl.ds((br * H + h) * NQB + qb0, XC // 128)] = jnp.stack(
                [blk[:, j * 128:(j + 1) * 128] for j in range(XC // 128)])

    def store_v(rows20, hidx, c0):
        vv = jnp.concatenate([rows20, jnp.ones((4, XC), F32)], axis=0)
        vt[hidx, pl.ds(c0, XC // 128), 0:24, :] = jnp.stack(
            [vv[:, j * 128:(j + 1) * 128] for j in range(XC // 128)])

    def proj_b(i):
        xc = bx[xrows(i), :]
        r = lax.dot_general(lhs_b[0:D + 48, :], xc, _NT, preferred_element_type=F32)
        store_q(r[48:48 + D], 1, i * (XC // 128))
        store_v(r[24:24 + DH], H, i * (XC // 128))
        k = jnp.concatenate([r[0:24], z(104, XC, F32)], axis=0).T.astype(BF16)
        kp[H, pl.ds(i * (XC // 2), XC // 2), :] = pltpu.bitcast(k, F32)

    c_bx[0].wait()
    c_bx[2].start()
    c_bx[3].start()
    proj_b(0)
    c_bx[1].wait()
    c_awqkv.start()
    proj_b(1)
    c_bx[2].wait()
    c_bx[3].wait()
    for k in range(NXC):
        c_ax[k].start()
    proj_b(2)
    c_awqkv.wait()
    prep_a()
    proj_b(3)
    for k in range(NXC):
        c_ax[k].wait()
    c_awo.start()
    c_bwo.start()

    lane = lax.broadcasted_iota(jnp.int32, (64, 128), 1)

    def proj_a(i, c):
        rows = pl.ds(pl.multiple_of(i * XC, XC), XC)
        xc = ax[rows, :]
        for j in range(XC // 128):
            k = jnp.dot(xc[j * 128:(j + 1) * 128], awqkv[:, D:2 * D], preferred_element_type=F32).astype(BF16)
            k = pltpu.bitcast(k, F32)
            for h in range(H):
                t, off = divmod(DH * h, 128)
                win = k[:, 128 * t:128 * (t + 1)]
                if off:
                    win = pltpu.roll(win, 128 - off, 1)
                if off + DH > 128:
                    nxt = pltpu.roll(k[:, 128 * (t + 1):128 * (t + 2)], 128 - off, 1)
                    win = jnp.where(lane < 128 - off, win, nxt)
                kp[h, pl.ds(pl.multiple_of(i * (XC // 2) + j * 64, 64), 64), :] = win
        r = lax.dot_general(lhs_a[...], xc, _NT, preferred_element_type=F32)
        store_q(r[0:D], 0, i * (XC // 128))
        for h in range(H):
            store_v(r[D + DH * h:D + DH * (h + 1)], h, i * (XC // 128))
        return c
    lax.fori_loop(0, NXC, proj_a, 0)

    def st(buf, r0, n, v, val):
        o = 0
        while o < n:
            c, rr = divmod(r0 + o, TK)
            k = min(n - o, TK - rr)
            buf[c][0, rr:rr + k, v * 128:(v + 1) * 128] = val[o:o + k]
            o += k

    def produce(kidx, kb, g, k, flag, gate):
        k32 = kp[kidx, 8 * g:8 * (g + 1), :]
        if gate is not None:
            k32 = jnp.where(flag, gate, k32)
        kf = pltpu.bitcast(k32, BF16).astype(F32)
        bc = [jnp.broadcast_to(kf[:, d:d + 1], (16, 128)) for d in range(k * DS, (k + 1) * DS)]
        for r in range(2):
            pr, a = divmod(2 * g + r, PK)
            kb[pr][k][0, a * DS:(a + 1) * DS] = jnp.stack([x[8 * r:8 * (r + 1)] for x in bc])

    class P1:
        def __init__(self, u, s, off):
            bh = u // 4
            self.bh = bh
            self.kidx = jnp.minimum(bh, H)
            qc = s % 4
            self.hs = s // 4
            self.off = off
            self.msz = MSZ if off else [TK] * NC
            self.moff = MOFF if off else [TK * c for c in range(NC)]
            q4 = qt[pl.ds(bh * NQB + qc * 4, 4)]
            self.qblk = [pltpu.bitcast(q4[v], BF16) for v in range(4)]
            self.w = [jnp.concatenate([b, z(96, 128, BF16)], axis=0) for b in self.qblk]
            self.mx = [None] * 4
            self.mv = [None] * 4
            self.buf = bufs[s % 2]
            self.qs = qss[s % 2]

        def build(self, v, r, d0, zoff, flag, gate):
            qs = self.qs[v]
            if r == 0 and d0 == 0:
                qf = self.qblk[v].astype(F32)
                rows = [jnp.broadcast_to(qf[d:d + 1], (8, 128)) for d in range(DH)]
                if gate is not None:
                    rows[0] = jnp.where(flag, gate, rows[0])
                qs[0] = jnp.stack(rows)
            n = min(PK, NV // 8 - r * PK)
            acc = self.acc if d0 else None
            kk = kbs[self.hs % 3][r][d0 // DS][zoff, 0:n * DS].reshape(n, DS, 8, 128)
            qq = qs[zoff, d0:d0 + DS]
            for i in range(DS):
                t = kk[:, i] * qq[i][None]
                acc = t if acc is None else acc + t
            self.acc = acc
            if d0 + DS == DH:
                st(self.buf, r * PK * 8, 8 * n, v, acc.reshape(8 * n, 128))
                am = jnp.max(acc, axis=0)
                self.mv[v] = am if self.mv[v] is None else jnp.maximum(self.mv[v], am)
            return [acc[j] for j in range(n)]

        def chunk(self, c, v, flag, anch):
            if v == 0:
                self.kc = kp[self.kidx, pl.ds(self.moff[c] // 2, self.msz[c] // 2), :]
            kc = self.kc
            if anch:
                parts = []
                for j in range(self.msz[c] // 16):
                    p32 = kc[8 * j:8 * (j + 1)]
                    for val in anch.get(j, []):
                        p32 = jnp.where(flag, val, p32)
                    parts.append(p32)
                kc = jnp.concatenate(parts, axis=0)
            s = jnp.dot(pltpu.bitcast(kc, BF16), self.w[v], preferred_element_type=F32)
            st(self.buf, self.moff[c], self.msz[c], v, s)
            mc = jnp.max(s.reshape(self.msz[c] // 8, 8, 128), axis=0)
            self.mx[v] = mc if self.mx[v] is None else jnp.maximum(self.mx[v], mc)
            return s[0:8]

        def finish(self, v):
            m = jnp.maximum(self.mx[v], self.mv[v]) if self.off else self.mx[v]
            return jnp.max(m, axis=0, keepdims=True)

    class P2:
        def __init__(self, u, qc, par, zoff):
            self.u = u
            self.bh = u // 4
            self.qc = qc
            self.vidx = jnp.minimum(self.bh, H)
            self.acc = [None] * 4
            self.buf, self.zoff = bufs[par], zoff

        def chunk(self, c, v, m):
            if v == 0:
                self.sc = self.buf[c][self.zoff]
            p = jnp.exp2(self.sc[:, v * 128:(v + 1) * 128] - m)
            if v == 0:
                self.vv = vt[self.vidx, c, 0:24, :]
            d = jnp.dot(self.vv, p, preferred_element_type=F32,
                        precision=lax.Precision.DEFAULT)
            self.acc[v] = d if self.acc[v] is None else self.acc[v] + d
            if c == NC - 1:
                a = self.acc[v]
                br, h = self.bh // H, self.bh % H
                ot[br * NQB + self.qc * 4 + v, pl.ds(pl.multiple_of(h * 24, 8), 24), :] = a

        def recip(self, flag, gate):
            row = lax.broadcasted_iota(jnp.int32, (8, 128), 0)
            l = self.acc[3][16:24]
            if gate is not None:
                l = jnp.where(flag, gate, l)
            for k in (2, 1, 0):
                l = jnp.where(row == 4 + k, self.acc[k][16:24], l)
            rls[self.u] = 1.0 / l

    def run(u0, s0, n1, n2, m, zoff, extra=()):
        ms = {}
        if m is not None:
            for v in range(4):
                ms[(0, v)] = m[:, v * 128:(v + 1) * 128]
        p1s, p2s = {}, {}
        lag = LJ if n1 else 0
        extra = list(extra)
        flag = (jnp.full((8, 128), zoff, jnp.int32) != 0) if n1 else None

        def getp1(t):
            if t not in p1s:
                p1s[t] = P1(u0 + t + 1, s0 + t + 1, s0 + t + 1 > 0)
            return p1s[t]

        njobs = n1 * NC * 4
        jt = lambda n: n * SLOT // 4
        nj = lambda n: (MSZ if s0 + n // (4 * NC) + 1 > 0 else [TK] * NC)[(n // 4) % NC] // 16
        pts = sorted((jt(n) + 16 * j, n, j) for n in range(njobs) for j in range(nj(n)))
        builds = {}
        anchors = {}
        gates = {}
        L = SLOT * NC
        later = {}
        last_prod = {}
        for t in range(n1):
            s = s0 + t + 1
            if s > 0:
                w = [p for p in pts if max(t * L + T0, TS) <= p[0] <= (t + 1) * L - T1]
                subs = [((v + CR) % 4, r, d0) for v in range(4) for r in range(NR) for d0 in range(0, DH, DS)]
                wt = [min(PK, NV // 8 - r * PK) for (v, r, d0) in subs]
                tot = sum(wt)
                mines = []
                pos = 0
                for n in wt:
                    mines.append([w[(pos + j) * len(w) // tot] for j in range(n)])
                    pos += n
                firsts = [min(p[1] for p in mine) for mine in mines]
                for k in range(len(firsts) - 2, -1, -1):
                    firsts[k] = min(firsts[k], firsts[k + 1])
                assert firsts[0] > last_prod.get(s // 4, -1)
                assert firsts[-1] <= (t + 1) * 4 * NC - 4
                for (v, r, d0), mine, first in zip(subs, mines, firsts):
                    gj = max([n for n in range(first) if jt(n) <= mine[0][0] - GD], default=None)

                    def bld(t=t, v=v, r=r, d0=d0, mine=mine, gj=gj):
                        vals = getp1(t).build(v, r, d0, zoff, flag, None if gj is None else gates[gj])
                        for val, p in zip(vals, mine):
                            anchors.setdefault(p[1], {}).setdefault(p[2], []).append(val)
                    builds.setdefault(first, []).append(bld)
            grp = [(s // 4 + 1, g, k) for g in range(X * (s % 4) // 4, X * (s % 4 + 1) // 4) for k in range(ND)]
            if s == 0:
                grp = [(0, g, k) for g in range(X) for k in range(ND)] + grp
            w = [p for p in pts if max(t * L + PS, TS + 100) <= p[0] <= (t + 1) * L - PE]
            for i, (hs, g, k) in enumerate(grp):
                p = w[(2 * i + 1) * len(w) // (2 * len(grp))]
                gj = max([n for n in range(p[1]) if jt(n) <= p[0] - PGD], default=None)

                def prod(t=t, hs=hs, g=g, k=k, p=p, s=s, gj=gj):
                    kidx = jnp.minimum(getp1(t).bh + (hs - s // 4), H)
                    produce(kidx, kbs[hs % 3], g, k, flag, None if gj is None else gates[gj])
                    pr, a = divmod(2 * g, PK)
                    val = kbs[hs % 3][pr][k][zoff, a * DS]
                    anchors.setdefault(p[1], {}).setdefault(p[2], []).append(val)
                builds.setdefault(p[1], []).append(prod)
                last_prod[hs] = max(last_prod.get(hs, -1), p[1])

        for n in range(max(njobs, n2 * NC * 4 + lag)):
            if n < njobs:
                t, c, vi = n // (4 * NC), (n // 4) % NC, n % 4
                for f in builds.get(n, []):
                    f()
                gates[n] = getp1(t).chunk(c, vi, flag, anchors.get(n))
                if c == NC - 1:
                    ms[(t + 1, vi)] = p1s[t].finish(vi)
            n_ = n - lag
            if 0 <= n_ < n2 * NC * 4:
                t, c, v = n_ // (4 * NC), (n_ // 4) % NC, n_ % 4
                if t not in p2s:
                    p2s[t] = P2(u0 + t, (s0 + t) % 4, (s0 + t) % 2, zoff)
                p2s[t].chunk(c, v, ms[(t, v)])
                if c == NC - 1 and v == 3:
                    if n + DJ < njobs:
                        later.setdefault(n + DJ, []).append(p2s[t])
                    else:
                        p2s[t].recip(None, None)
            for p2 in later.get(n, []):
                p2.recip(flag, gates[n])
            if extra and n % 4 == 3:
                extra.pop(0)()
        for f in extra:
            f()
        if n1:
            return jnp.concatenate([ms[(n1, v)] for v in range(4)], axis=1)

    zoff0 = zero_ref[0]
    m0 = run(-1, -1, 1, 0, None, zoff0)
    m0 = run(0, 0, NPRE, NPRE, m0, zoff0)

    def body(i, m):
        return run(NPRE + i * NH, NPRE, NH, NH, m, zero_ref[0])
    m_last = lax.fori_loop(0, (NU - 1 - NPRE) // NH, body, m0)

    c_awo.wait()
    c_bwo.wait()

    def ocopy(i):
        rows = pl.ds(OCH[i][0] * 128, OCH[i][1] * 128)
        return pltpu.make_async_copy(outv.at[rows], out_h.at[rows], osem.at[i])

    def o_t(br, qb):
        o24 = ot[br * NQB + qb]
        rl = lambda h: rls[(br * H + h) * 4 + qb // 4, 4 + qb % 4:5 + qb % 4, :]
        return jnp.concatenate([o24[24 * h:24 * h + DH] * rl(h) for h in range(H)], axis=0).astype(BF16)

    def oproj(i):
        rows = pl.ds(OCH[i][0] * 128, OCH[i][1] * 128)
        for br, wo in ((0, awo), (1, bwo)):
            o = jnp.concatenate([o_t(br, OCH[i][0] + j) for j in range(OCH[i][1])], axis=1)
            res = lax.dot_general(o, wo[...], _TN, preferred_element_type=F32)
            outv[rows, br * D:(br + 1) * D] = res.astype(BF16)
        ocopy(i).start()

    pieces = []
    for br, wo in ((0, awo), (1, bwo)):
        for j in range(OCH[0][1]):
            o_n = o_t(br, j).T
            for n in range(D // 128):
                def piece(br=br, wo=wo, j=j, n=n, o_n=o_n):
                    res = jnp.dot(o_n, wo[:, n * 128:(n + 1) * 128], preferred_element_type=F32)
                    outv[j * 128:(j + 1) * 128, br * D + n * 128:br * D + (n + 1) * 128] = res.astype(BF16)
                pieces.append(piece)
    run(NU - 1, 3, 0, 1, m_last, 0, extra=pieces)
    ocopy(0).start()
    for i in range(1, NOC):
        oproj(i)
    for i in range(NOC):
        ocopy(i).wait()


@jax.jit
def pallas_concat_heads__softmax_full_mha__grouped_kv_mqa__prompt_kernel(
    A_x: jax.Array,
    A_wqkv: jax.Array,
    A_wo: jax.Array,
    B_x: jax.Array,
    B_wq: jax.Array,
    B_wk: jax.Array,
    B_wv: jax.Array,
    B_wo: jax.Array,
):
    anyspec = pl.BlockSpec(memory_space=pl.ANY)
    scratch = [
        pltpu.VMEM((S, D), BF16),
        pltpu.VMEM((D, 3 * D), BF16),
        pltpu.VMEM((D, D), BF16),
        pltpu.VMEM((S, D), BF16),
        pltpu.VMEM((D, D), BF16),
        pltpu.VMEM((D, D), BF16),
        pltpu.VMEM((S, 2 * D), BF16),
        pltpu.VMEM((2 * D, D), BF16),
        pltpu.VMEM((D + 64, D), BF16),
        pltpu.VMEM((H + 1, S // 2, 128), F32),
        pltpu.VMEM((2 * H * NQB, 16, 128), F32),
        pltpu.VMEM((H + 1, NC, 32, 128), F32),
        pltpu.VMEM((2 * NQB, H * 24, 128), F32),
        pltpu.VMEM((NU, 8, 128), F32),
        pltpu.SMEM((1,), jnp.int32),
        pltpu.SemaphoreType.DMA((14,)),
        pltpu.SemaphoreType.DMA((NOC,)),
    ]
    scratch += [pltpu.VMEM((1, KBN, 8, 128), F32)] * (3 * NR * ND)
    scratch += [pltpu.VMEM((1, DH, 8, 128), F32)] * 8
    scratch += [pltpu.VMEM((1, TK, 512), F32)] * (2 * NC)
    scratch += [pltpu.VMEM((DH, D), BF16)] * 2
    out = pl.pallas_call(
        _kernel,
        out_shape=jax.ShapeDtypeStruct((S, 2 * D), BF16),
        in_specs=[anyspec] * 8,
        out_specs=anyspec,
        scratch_shapes=scratch,
        compiler_params=pltpu.CompilerParams(vmem_limit_bytes=110 * 1024 * 1024),
        name="mha_mqa",
    )(A_x.reshape(S, D), A_wqkv, A_wo, B_x.reshape(S, D), B_wq, B_wk.T, B_wv.T, B_wo)
    return out.reshape(1, S, 2 * D)
```
